```python
import jax
import jax.numpy as jnp

def _softmax(x, axis=-1):
    return jax.nn.softmax(x, axis=axis)
def _gelu(x):
    return jax.nn.gelu(x, approximate=True)
def _silu(x):
    return jax.nn.silu(x)
def _sigmoid(x):
    return jax.nn.sigmoid(x)
def _layernorm(x, axis=-1, eps=1e-5):
    m = jnp.mean(x, axis=axis, keepdims=True)
    v = jnp.var(x, axis=axis, keepdims=True)
    return (x - m) / jnp.sqrt(v + eps)
def _scatter_add(tgt, idx, src, axis=0):
    return tgt.at[idx].add(src)
def _segment_sum(src, seg, n):
    return jax.ops.segment_sum(src, seg, n)
class _Rng:
    def __init__(self, key):
        self._k = key
    def _next(self):
        self._k, sub = jax.random.split(self._k)
        return sub
    def normal(self, shape):
        return jax.random.normal(self._next(), shape, dtype=jnp.bfloat16)
    def randint(self, lo, hi, shape):
        return jax.random.randint(self._next(), shape, lo, hi, dtype=jnp.int32)
    def uniform(self, shape, lo=0.0, hi=1.0):
        return jax.random.uniform(self._next(), shape, jnp.bfloat16, lo, hi)
    def permutation(self, n):
        return jax.random.permutation(self._next(), n)


kernel_name = 'recurrent_scan__mha_block_cached__moe_arch_mod__prompt'

def setup_inputs():
    _rng = _Rng(jax.random.key(int.from_bytes(__import__("os").urandom(4), "little")))
    _w = (lambda a: (lambda t: t.astype(jnp.bfloat16) if jnp.issubdtype(t.dtype, jnp.floating) else t)(jnp.asarray(a)))
    def _A_setup():
        B, Sq, D = 1, 2048, 640
        H, Sk, Dh = 32, 2048, 128
        return {
            "x": _w((lambda *s: _rng.normal(s) * 0.05)(B, Sq, D)),
            "k_cache": _w((lambda *s: _rng.normal(s) * 0.05)(B, H, Sk, Dh)),
            "v_cache": _w((lambda *s: _rng.normal(s) * 0.05)(B, H, Sk, Dh)),
            "wq": _w((lambda *s: _rng.normal(s) * 0.05)(D, H * Dh) * (D ** -0.5)),
            "wo": _w((lambda *s: _rng.normal(s) * 0.05)(H * Dh, D) * ((H * Dh) ** -0.5)),
        }
    _A_in = _A_setup()

    def _B_setup():
        B, S, D, F, C = 1, 2048, 640, 1728, 8
        return {
            "x": _w((lambda *s: _rng.normal(s) * 0.05)(B, S, D)),
            "w_r": _w((lambda *s: _rng.normal(s) * 0.05)(D)),
            "w_gate": _w((lambda *s: _rng.normal(s) * 0.05)(D, F)),
            "w_up": _w((lambda *s: _rng.normal(s) * 0.05)(D, F)),
            "w_down": _w((lambda *s: _rng.normal(s) * 0.05)(F, D)),
        }
    _B_in = _B_setup()

    return {
        "A_x": _A_in["x"],
        "A_k_cache": _A_in["k_cache"],
        "A_v_cache": _A_in["v_cache"],
        "A_wq": _A_in["wq"],
        "A_wo": _A_in["wo"],
        "B_x": _B_in["x"],
        "B_w_r": _B_in["w_r"],
        "B_w_gate": _B_in["w_gate"],
        "B_w_up": _B_in["w_up"],
        "B_w_down": _B_in["w_down"],
    }

def reference(A_x, A_k_cache, A_v_cache, A_wq, A_wo, B_x, B_w_r, B_w_gate, B_w_up, B_w_down):
    def _A_ref(x, k_cache, v_cache, wq, wo):
        B, Sq, D = x.shape
        H, Dh = 32, 128
        q = (lambda x, *d: x.transpose(*d))((x @ wq).reshape(B, Sq, H, Dh), 0, 2, 1, 3)
        scores = jnp.einsum("bhqd,bhkd->bhqk", q, k_cache) * (Dh ** -0.5)
        p = _softmax(scores, axis=-1)
        o = jnp.einsum("bhqk,bhkd->bhqd", p, v_cache)
        return (lambda x, *d: x.transpose(*d))(o, 0, 2, 1, 3).reshape(B, Sq, H * Dh) @ wo

    def _B_ref(x, w_r, w_gate, w_up, w_down):
        B, S, D = x.shape
        C = 8
        r = x @ w_r
        idx = jnp.argsort(-r, axis=-1)[:, :C]
        idx_e = jnp.repeat(idx.reshape(B, C, 1), D, axis=2)
        x_sel = jnp.take_along_axis(x, idx_e, axis=1)
        g = _silu(x_sel @ w_gate)
        u = x_sel @ w_up
        y = (g * u) @ w_down
        r_sel = _sigmoid(jnp.take_along_axis(r, idx, axis=1))
        y = y * r_sel.reshape(B, C, 1)
        b_off = (jnp.arange(B) * S).reshape(B, 1)
        flat_idx = (idx + b_off).reshape(B * C)
        zero = (x * 0.0).reshape(B * S, D)
        upd = _scatter_add(zero, flat_idx, y.reshape(B * C, D), axis=0)
        return x + upd.reshape(B, S, D)

    x = A_x
    xn = _layernorm(x, axis=-1)
    s = _A_ref(xn, A_k_cache, A_v_cache, A_wq, A_wo)
    g = _silu(_B_ref(xn, B_w_r, B_w_gate, B_w_up, B_w_down))
    return x + s * g
```

```python
import functools
import math

import jax
import jax.numpy as jnp
from jax import lax
import jax.experimental.pallas as pl
import jax.experimental.pallas.tpu as pltpu

F32 = jnp.float32
BF16 = jnp.bfloat16
I32 = jnp.int32

H, DH = 32, 128
CAP = 8
EPS = 1e-5
NT = (((1,), (1,)), ((), ()))


def _bf(x):
    return x.astype(BF16).astype(F32)


def _silu(x):
    h = 0.5 * x
    return h + h * jnp.tanh(h)


def _layernorm(x):
    d = x.shape[-1]
    x = x.astype(F32)
    mu = jnp.sum(x, axis=-1, keepdims=True) * (1.0 / d)
    xc = x - mu
    var = jnp.sum(xc * xc, axis=-1, keepdims=True) * (1.0 / d)
    den = _bf(jnp.sqrt(_bf(_bf(var) + _bf(jnp.full_like(var, EPS)))))
    inv = pl.reciprocal(den, approx=True)
    inv = jnp.where(den == jnp.inf, 0.0, inv * (2.0 - den * inv))
    return (_bf(x - _bf(mu)) * inv).astype(BF16)


def _attend(nb, ng, lhs, wq, keys, vals, wo, acc_in, emit, q_ref, cfg):
    R, CK, lead = cfg["R"], cfg["CK"], cfg["lead"]
    nck = cfg["Sk"] // CK
    qscale = (DH ** -0.5) * math.log2(math.e)
    st = {}

    def proj_q(b):
        q = jnp.dot(lhs(b), wq(), preferred_element_type=F32)
        q_ref[b, :, :ng * DH] = (q * qscale).astype(BF16)

    def scores(u, c):
        b, h = divmod(u, ng)
        if c == 0:
            st["q", u] = q_ref[b, :, h * DH:(h + 1) * DH]
        s = lax.dot_general(st["q", u], keys(h, c), NT, preferred_element_type=F32)
        st["s", u, c] = s
        m = s[:, :128]
        if c > 0:
            m = jnp.maximum(m, st["m", u])
        for j in range(1, CK // 128):
            m = jnp.maximum(m, s[:, j * 128:(j + 1) * 128])
        if c == nck - 1:
            m = jnp.broadcast_to(jnp.max(m, axis=-1, keepdims=True), (R, 128))
        st["m", u] = m

    def values(u, c):
        b, h = divmod(u, ng)
        p = jnp.exp2(st["s", u, c] - jnp.concatenate([st["m", u]] * (CK // 128), axis=1))
        l = p[:, :128]
        if c > 0:
            l = l + st["l", u]
        for j in range(1, CK // 128):
            l = l + p[:, j * 128:(j + 1) * 128]
        st["l", u] = l
        p = jnp.concatenate([p[:, :CK - 128], jnp.minimum(p[:, CK - 128:], l)], axis=1)
        o = jnp.dot(p.astype(BF16), vals(h, c), preferred_element_type=F32)
        st["o", u] = o if c == 0 else o + st["o", u]
        if c == nck - 1:
            l = jnp.sum(l, axis=-1, keepdims=True)
            r = pl.reciprocal(l, approx=True)
            st["o", u] = st["o", u] * (r * (2.0 - l * r))

    def proj_o(b, split):
        a = acc_in(b)
        for h0, h1 in ([(0, ng - 1), (ng - 1, ng)] if split else [(0, ng)]):
            o = jnp.concatenate([st["o", b * ng + h] for h in range(h0, h1)], axis=1).astype(BF16)
            y = jnp.dot(o, wo(h0, h1), preferred_element_type=F32)
            a = y if a is None else y + a
        emit(b, a)

    prog = []
    for j in range(nb * ng * nck):
        prog.append(((j - lead, 1), scores, divmod(j, nck)))
        prog.append(((j, 3), values, divmod(j, nck)))
    for b in range(nb):
        prog.append(((b * ng * nck - lead - cfg["apos"], 4), proj_q, (b,)))
        prog.append((((b + 1) * ng * nck + cfg["epos"], 4), proj_o, (b, b == nb - 1 and ng > 1)))
    for _, fn, args in sorted(prog, key=lambda e: e[0]):
        fn(*args)


def _kernel(x_hbm, k_hbm, v_hbm, wq_hbm, wo_hbm, wr_hbm, wg_hbm, wu_hbm, wd_hbm, out_hbm,
            x_ref, xn_ref, upd_ref, acc_ref, out_ref, k_ref, v_ref, wq0_ref, wq1_ref, wo_ref,
            wgu_ref, gu_ref, wd_ref, q0_ref, q1_ref, score_ref, top_ref, wr_ref,
            x_sem, w_sem, p_sem, o_sem, *, cfg):
    S, D = x_ref.shape
    R, CK = cfg["R"], cfg["CK"]
    n0, ng, nb0, nb1 = cfg["n0"], cfg["ng"], cfg["nb0"], cfg["nb1"]
    n1 = (H - n0) // ng
    parts0, parts1 = S // (nb0 * R), S // (nb1 * R)

    def pass_copies(idx, h0, n, wq_dst):
        w0 = h0 * DH if isinstance(h0, int) else pl.multiple_of(h0 * DH, DH)
        return [
            pltpu.make_async_copy(wq_hbm.at[:, pl.ds(w0, n * DH)], wq_dst, p_sem.at[idx, 0]),
            pltpu.make_async_copy(k_hbm.at[0, pl.ds(h0, n)], k_ref.at[pl.ds(h0, n)], p_sem.at[idx, 1]),
            pltpu.make_async_copy(v_hbm.at[0, pl.ds(h0, n)], v_ref.at[pl.ds(h0, n)], p_sem.at[idx, 2]),
            pltpu.make_async_copy(wo_hbm.at[pl.ds(w0, n * DH)], wo_ref.at[pl.ds(w0, n * DH)], p_sem.at[idx, 3]),
        ]

    def x_copy(part):
        start = part * (nb0 * R)
        rows = pl.ds(start if isinstance(part, int) else pl.multiple_of(start, nb0 * R), nb0 * R)
        return pltpu.make_async_copy(x_hbm.at[0, rows], x_ref.at[rows], x_sem.at[part])

    def out_copy(part):
        start = part * (nb1 * R)
        rows = pl.ds(start if isinstance(part, int) else pl.multiple_of(start, nb1 * R), nb1 * R)
        return pltpu.make_async_copy(out_ref.at[rows], out_hbm.at[0, rows], o_sem.at[part])

    single = lambda h: pass_copies(h, h, 1, wq0_ref.at[h])
    group = lambda g: pass_copies(n0 + g, n0 + g * ng, ng, wq1_ref.at[g])
    wr_copy = pltpu.make_async_copy(wr_hbm, wr_ref, w_sem.at[0])
    ffn_copies = [pltpu.make_async_copy(src, dst, w_sem.at[i + 1])
                  for i, (src, dst) in enumerate([(wg_hbm, wgu_ref.at[0]), (wu_hbm, wgu_ref.at[1]), (wd_hbm, wd_ref)])]

    def start(copies):
        for c in copies:
            c.start()

    def wait(copies):
        for c in copies:
            c.wait()

    def head_refs(h0):
        w0 = pl.multiple_of(h0 * DH, DH)
        return (lambda h, c: k_ref[h0 + h, c * CK:(c + 1) * CK, :],
                lambda h, c: v_ref[h0 + h, c * CK:(c + 1) * CK, :],
                lambda a, b: wo_ref[pl.ds(w0 + a * DH, (b - a) * DH), :])

    lane = lax.broadcasted_iota(I32, (8, 128), 1)
    per_part = nb0 * R // 8

    def norm_part(part):
        rows = pl.ds(pl.multiple_of(part * (nb0 * R), nb0 * R), nb0 * R)
        xn = _layernorm(x_ref[rows, :])
        xn_ref[rows, :] = xn
        r = jnp.sum(xn.astype(F32) * wr_ref[...].astype(F32).reshape(1, D), axis=-1, keepdims=True)
        score = jnp.broadcast_to(r[:8], (8, 128))
        for j in range(1, per_part):
            score = jnp.where(lane % per_part == j, r[j * 8:(j + 1) * 8], score)
        score_ref[part] = score

    def route():
        tiles = []
        for t in range(S // 1024):
            ps = range(t * (128 // per_part), (t + 1) * (128 // per_part))
            tile = score_ref[ps[0]]
            for j, p in enumerate(ps[1:]):
                tile = jnp.where(lane // per_part == j + 1, score_ref[p], tile)
            tiles.append(tile)
        r = _bf(jnp.concatenate(tiles, axis=1))
        r = jnp.where(r == 0.0, 0.0, r)
        bits = pltpu.bitcast(r, I32) >> 16
        rank = jnp.where(r != r, 0, jnp.where(bits < 0, ~bits, bits + 0x8000))
        token = lax.broadcasted_iota(I32, r.shape, 1) * 8 + lax.broadcasted_iota(I32, r.shape, 0)
        key = pltpu.bitcast(((rank << 11) | (S - 1 - token)) + 0x08000000, F32)
        slot = lax.broadcasted_iota(I32, (CAP, 128), 0)
        top = jnp.zeros((CAP, 128), F32)
        for c in range(CAP):
            best = jnp.max(jnp.max(key, axis=0, keepdims=True), axis=1, keepdims=True)
            top = jnp.where(slot == c, best, top)
            key = jnp.where(key == best, 0.0, key)
        top_ref[...] = pltpu.bitcast(top, I32) - 0x08000000

    def routed_ffn():
        wait(ffn_copies)
        top = top_ref[...]
        rank = top >> 11
        r_sel = pltpu.bitcast(jnp.where(rank < 0x8000, ~rank, rank - 0x8000) << 16, F32)
        picked = [(S - 1) - (top[c, 0] & (S - 1)) for c in range(CAP)]
        row = lax.broadcasted_iota(I32, (16, D), 0)
        slot = lax.broadcasted_iota(I32, (CAP, D), 0)
        xs = jnp.zeros((CAP, D), F32)
        for c, t in enumerate(picked):
            near = xn_ref[pl.ds(pl.multiple_of((t >> 4) << 4, 16), 16), :].astype(F32)
            xs = jnp.where(slot == c, jnp.sum(jnp.where(row == (t & 15), near, 0.0), axis=0, keepdims=True), xs)

        @pl.loop(0, 2)
        def _(j):
            gu_ref[j] = _bf(lax.dot_general(xs.astype(BF16), wgu_ref[j], NT, preferred_element_type=F32))

        g, u = gu_ref[0], gu_ref[1]
        y = _bf(jnp.dot((_bf(_silu(g)) * u).astype(BF16), wd_ref[...], preferred_element_type=F32))
        y = _bf(y * _bf(jax.nn.sigmoid(r_sel[:, :1])))
        for c, t in enumerate(picked):
            upd_ref[pl.ds(t, 1), :] = y[c:c + 1, :]

    start([wr_copy, x_copy(0)] + single(0))

    @pl.loop(0, S // 128)
    def _(i):
        upd_ref[pl.ds(pl.multiple_of(i * 128, 128), 128), :] = jnp.zeros((128, D), F32)

    score_ref[...] = jnp.zeros_like(score_ref)
    wr_copy.wait()

    def single_step(i, carry):
        h, part = i // parts0, i % parts0

        @pl.when(h == 0)
        def _():
            x_copy(part).wait()
            norm_part(part)

        @pl.when(part == 0)
        def _():
            wait(single(h))

        @pl.when(i == 0)
        def _():
            start([x_copy(p) for p in range(1, parts0)])

        @pl.when(i == 1)
        def _():
            for j in range(1, n0):
                start(single(j))
            start(group(0))

        rows = lambda b: pl.ds(pl.multiple_of(part * (nb0 * R), nb0 * R) + b * R, R)
        route()

        def store(b, a):
            acc_ref[rows(b), :] = a

        _attend(nb0, 1, lambda b: xn_ref[rows(b), :], lambda: wq0_ref[h], *head_refs(h),
                lambda b: jnp.where(h > 0, acc_ref[rows(b), :], 0.0), store, q0_ref, dict(cfg, **cfg["c0"]))
        return carry

    lax.fori_loop(0, n0 * parts0, single_step, 0)

    def group_step(i, carry):
        g, part = i // parts1, i % parts1

        @pl.when(part == 0)
        def _():
            wait(group(g))

            @pl.when(g < n1 - 1)
            def _():
                start(group(g + 1))

        @pl.when(i == 0)
        def _():
            start(ffn_copies)

        @pl.when(i == (n1 - 1) * parts1)
        def _():
            routed_ffn()

        rows = lambda b: pl.ds(pl.multiple_of(part * (nb1 * R), nb1 * R) + b * R, R)

        def store(b, a):
            acc_ref[rows(b), :] = a
            gate = _silu(xn_ref[rows(b), :].astype(F32) + upd_ref[rows(b), :])
            out_ref[rows(b), :] = (x_ref[rows(b), :].astype(F32) + a * gate).astype(out_ref.dtype)

        _attend(nb1, ng, lambda b: xn_ref[rows(b), :], lambda: wq1_ref[g], *head_refs(n0 + g * ng),
                lambda b: acc_ref[rows(b), :], store, q1_ref, cfg)

        @pl.when(g == n1 - 1)
        def _():
            out_copy(part).start()

        return carry

    if not cfg['skipm']: lax.fori_loop(0, n1 * parts1, group_step, 0)
    wait([out_copy(p) for p in range(parts1)])


def make(R=64, CK=512, lead=6, apos=3, epos=3, n0=2, ng=10, nb0=8, nb1=8, c0=dict(apos=9, epos=5), skipm=False, flags=None):
    @jax.jit
    def fn(A_x, A_k_cache, A_v_cache, A_wq, A_wo, B_x, B_w_r, B_w_gate, B_w_up, B_w_down):
        B, S, D = A_x.shape
        Sk = A_k_cache.shape[2]
        Fd = B_w_gate.shape[1]
        cfg = dict(R=R, CK=CK, lead=lead, apos=apos, epos=epos, n0=n0, ng=ng, nb0=nb0, nb1=nb1, c0=c0, skipm=skipm, Sk=Sk)
        n1 = (H - n0) // ng
        hbm = pl.BlockSpec(memory_space=pltpu.HBM)
        vmem, dma = pltpu.VMEM, pltpu.SemaphoreType.DMA
        return pl.pallas_call(
            functools.partial(_kernel, cfg=cfg),
            in_specs=[hbm] * 9,
            out_specs=hbm,
            out_shape=jax.ShapeDtypeStruct((B, S, D), A_x.dtype),
            scratch_shapes=[
                vmem((S, D), BF16), vmem((S, D), BF16), vmem((S, D), F32), vmem((S, D), F32), vmem((S, D), A_x.dtype),
                vmem((H, Sk, DH), BF16), vmem((H, Sk, DH), BF16),
                vmem((n0, D, DH), BF16), vmem((n1, D, ng * DH), BF16), vmem((H * DH, D), BF16),
                vmem((2, Fd, D), BF16), vmem((2, CAP, Fd), F32), vmem((Fd, D), BF16),
                vmem((nb0, R, DH), BF16), vmem((nb1, R, ng * DH), BF16),
                vmem((S // (nb0 * R), 8, 128), F32), vmem((CAP, 128), I32), vmem((D,), BF16),
                dma((S // (nb0 * R),)), dma((4,)), dma((n0 + n1, 4)), dma((S // (nb1 * R),)),
            ],
            compiler_params=pltpu.CompilerParams(vmem_limit_bytes=100 * 1024 * 1024, internal_scratch_in_bytes=64 * 1024, flags=flags),
        )(A_x, A_k_cache, A_v_cache, A_wq, A_wo, B_w_r, B_w_gate.T, B_w_up.T, B_w_down)
    return fn


pallas_recurrent_scan__mha_block_cached__moe_arch_mod__prompt_kernel = make()
```

```python
import functools
import math

import jax
import jax.numpy as jnp
from jax import lax
import jax.experimental.pallas as pl
import jax.experimental.pallas.tpu as pltpu

F32 = jnp.float32
BF16 = jnp.bfloat16
I32 = jnp.int32

H, DH = 32, 128
CAP = 8
EPS = 1e-5
NT = (((1,), (1,)), ((), ()))
QW = 8 * DH


def _bf(x):
    return x.astype(BF16).astype(F32)


def _silu(x):
    h = 0.5 * x
    return h + h * jnp.tanh(h)


def _after(x, other, zero):
    bits = pltpu.bitcast(x, I32) | (pltpu.bitcast(other, I32) & jnp.full(x.shape, zero, I32))
    return pltpu.bitcast(bits, F32)


def _layernorm(x, pace=None):
    d = x.shape[-1]
    x = x.astype(F32)
    if pace is not None:
        x = jnp.concatenate([_after(x[:, :128], *pace), x[:, 128:]], axis=1)
    mu = jnp.sum(x, axis=-1, keepdims=True) * (1.0 / d)
    xc = x - mu
    var = jnp.sum(xc * xc, axis=-1, keepdims=True) * (1.0 / d)
    den = _bf(jnp.sqrt(_bf(_bf(var) + _bf(jnp.full_like(var, EPS)))))
    inv = pl.reciprocal(den, approx=True)
    inv = jnp.where(den == jnp.inf, 0.0, inv * (2.0 - den * inv))
    return (_bf(x - _bf(mu)) * inv).astype(BF16)


def _attend(nb, ng, query, keys, vals, wo, acc_in, emit, cfg):
    R, CK, lead, eg = cfg["R"], cfg["CK"], cfg["lead"], cfg["eg"]
    nck = cfg["Sk"] // CK
    st = {}

    def scores(u, c):
        b, h = divmod(u, ng)
        if c == 0:
            st["q", u] = query(b, h)
        s = lax.dot_general(st["q", u], keys(h, c), NT, preferred_element_type=F32)
        st["s", u, c] = s
        m = s[:, :128]
        if c > 0:
            m = jnp.maximum(m, st["m", u])
        for j in range(1, CK // 128):
            m = jnp.maximum(m, s[:, j * 128:(j + 1) * 128])
        if c == nck - 1:
            m = jnp.broadcast_to(jnp.max(m, axis=-1, keepdims=True), (R, 128))
        st["m", u] = m

    def values(u, c):
        b, h = divmod(u, ng)
        p = jnp.exp2(st["s", u, c] - jnp.concatenate([st["m", u]] * (CK // 128), axis=1))
        l = p[:, :128]
        if c > 0:
            l = l + st["l", u]
        for j in range(1, CK // 128):
            l = l + p[:, j * 128:(j + 1) * 128]
        st["l", u] = l
        p = jnp.concatenate([p[:, :CK - 128], jnp.minimum(p[:, CK - 128:], l)], axis=1)
        o = jnp.dot(p.astype(BF16), vals(h, c), preferred_element_type=F32)
        st["o", u] = o if c == 0 else o + st["o", u]
        if c == nck - 1:
            l = jnp.sum(l, axis=-1, keepdims=True)
            r = pl.reciprocal(l, approx=True)
            st["o", u] = st["o", u] * (r * (2.0 - l * r))

    def project(b, h0, h1):
        o = jnp.concatenate([st["o", b * ng + h] for h in range(h0, h1)], axis=1).astype(BF16)
        a = acc_in(b) if h0 == 0 else st["a", b]
        st["a", b] = jnp.dot(o, wo(h0, h1), preferred_element_type=F32) + a
        if h1 == ng:
            emit(b, st["a", b])

    prog = []
    for j in range(nb * ng * nck):
        prog.append(((j - lead, 1), scores, divmod(j, nck)))
        prog.append(((j, 3), values, divmod(j, nck)))
    for b in range(nb):
        cuts = list(range(0, ng, eg)) + [ng]
        if b == nb - 1:
            cuts[-1:] = [ng - 1, ng]
        for h0, h1 in zip(cuts, cuts[1:]):
            late = cfg["epos"] if h1 % eg == 0 else cfg["elast"]
            prog.append((((b * ng + h1) * nck + late, 4), project, (b, h0, h1)))
    for _, fn, args in sorted(prog, key=lambda e: e[0]):
        fn(*args)


def _kernel(x_hbm, k_hbm, v_hbm, wq_hbm, wo_hbm, wr_hbm, wg_hbm, wu_hbm, wd_hbm, out_hbm,
            x_ref, xn_ref, upd_ref, acc_ref, out_ref, q_ref, k_ref, v_ref, wq_ref, wo_ref,
            wg_ref, wu_ref, wd_ref, xs_ref, head_ref, score_ref, top_ref, wr_ref,
            x_sem, q_sem, w_sem, p_sem, o_sem, *, cfg):
    S, D = x_ref.shape
    F = wg_hbm.shape[0]
    R, CK, ng, nb = cfg["R"], cfg["CK"], cfg["ng"], cfg["nb"]
    R0, P0, R1, P1, FC = cfg["R0"], cfg["P0"], cfg["R1"], cfg["P1"], cfg["FC"]
    panels, groups = H * DH // QW, H // ng
    parts0, parts1, parts2 = S // P0, S // P1, S // (nb * R)
    qscale = (DH ** -0.5) * math.log2(math.e)

    def span(i, n):
        return pl.ds(i * n if isinstance(i, int) else pl.multiple_of(i * n, n), n)

    def x_copy(i):
        return pltpu.make_async_copy(x_hbm.at[0, span(i, P0)], x_ref.at[span(i, P0)], x_sem.at[i])

    def wq_copy(i):
        return pltpu.make_async_copy(wq_hbm.at[:, span(i, QW)], wq_ref.at[i], q_sem.at[i])

    def group_copies(g):
        return [pltpu.make_async_copy(k_hbm.at[0, span(g, ng)], k_ref.at[span(g, ng)], p_sem.at[g, 0]),
                pltpu.make_async_copy(v_hbm.at[0, span(g, ng)], v_ref.at[span(g, ng)], p_sem.at[g, 1]),
                pltpu.make_async_copy(wo_hbm.at[span(g, ng * DH)], wo_ref.at[span(g, ng * DH)], p_sem.at[g, 2])]

    def out_copy(i):
        return pltpu.make_async_copy(out_ref.at[span(i, nb * R)], out_hbm.at[0, span(i, nb * R)], o_sem.at[i])

    wr_copy = pltpu.make_async_copy(wr_hbm, wr_ref, w_sem.at[0])
    ffn_copies = [pltpu.make_async_copy(src, dst.at[:F], w_sem.at[i + 1])
                  for i, (src, dst) in enumerate([(wg_hbm, wg_ref), (wu_hbm, wu_ref), (wd_hbm, wd_ref)])]

    def start(copies):
        for c in copies:
            c.start()

    def wait(copies):
        for c in copies:
            c.wait()

    def project_q(xn, panel, rows, half):
        cols = slice(half * QW // 2, (half + 1) * QW // 2)
        q = jnp.dot(xn, wq_ref[panel, :, cols], preferred_element_type=F32)
        q_ref[panel, rows, cols] = (q * qscale).astype(BF16)
        return q

    start([x_copy(0), wr_copy, wq_copy(0)])
    for ref in (wg_ref, wu_ref, wd_ref):
        ref[F:, :] = jnp.zeros((ref.shape[0] - F, D), BF16)
    xs_ref[...] = jnp.zeros_like(xs_ref)
    wait([x_copy(0)])
    head_ref[...] = _layernorm(x_ref[:R0, :])
    wait([wr_copy, wq_copy(0)])
    start([x_copy(i) for i in range(1, parts0)] + [wq_copy(1)])

    lane = lax.broadcasted_iota(I32, (8, 128), 1)
    per_part = P0 // 8

    def norm_step(i, carry):
        @pl.when(i < parts0 - 1)
        def _():
            x_copy(i + 1).wait()

        @pl.when(i == 1)
        def _():
            start(ffn_copies + [wq_copy(j) for j in range(2, panels)])

        wr = wr_ref[...].astype(F32).reshape(1, D)
        score = jnp.zeros((8, 128), F32)
        late, done = [], []
        pace = lambda b: (done[2 * b - cfg['pa']][:, cfg['pc'] * 128:(cfg['pc'] + 1) * 128], i >> 8) if 2 * b >= cfg['pa'] else None
        for b in range(P0 // R0):
            rows = span(i * (P0 // R0) + b, R0)
            xn = head_ref[...] if b == 0 else _layernorm(x_ref[rows, :], pace(b))
            if "n" in cfg["x"]: late.append((rows, xn))
            else: xn_ref[rows, :] = xn
            r = jnp.sum(xn.astype(F32) * wr, axis=-1, keepdims=True) if 'r' not in cfg['x'] else xn.astype(F32)[:, :128]
            for j in range(R0 // 8):
                score = jnp.where(lane % per_part == b * (R0 // 8) + j, r[j * 8:(j + 1) * 8], score)
            if "u" in cfg["x"]: upd_ref[rows, :] = jnp.zeros((R0, D), F32)
            done.append(project_q(xn, 0, rows, 0))
            done.append(project_q(xn, 0, rows, 1))
        score_ref[i] = score
        for rows, xn in late: xn_ref[rows, :] = xn
        ahead = jnp.minimum(i + 1, parts0 - 1) * (P0 // R0)
        head_ref[...] = _layernorm(x_ref[span(ahead, R0), :], pace(P0 // R0))
        return carry

    lax.fori_loop(0, parts0, norm_step, 0)

    def route():
        tiles = []
        for t in range(S // 1024):
            ps = range(t * (128 // per_part), (t + 1) * (128 // per_part))
            tile = score_ref[ps[0]]
            for j, p in enumerate(ps[1:]):
                tile = jnp.where(lane // per_part == j + 1, score_ref[p], tile)
            tiles.append(tile)
        r = _bf(jnp.concatenate(tiles, axis=1))
        r = jnp.where(r == 0.0, 0.0, r)
        bits = pltpu.bitcast(r, I32) >> 16
        rank = jnp.where(r != r, 0, jnp.where(bits < 0, ~bits, bits + 0x8000))
        token = lax.broadcasted_iota(I32, r.shape, 1) * 8 + lax.broadcasted_iota(I32, r.shape, 0)
        key = pltpu.bitcast(((rank << 11) | (S - 1 - token)) + 0x08000000, F32)
        slot = lax.broadcasted_iota(I32, (CAP, 128), 0)
        top = jnp.zeros((CAP, 128), F32)
        for c in range(CAP):
            best = jnp.max(jnp.max(key, axis=0, keepdims=True), axis=1, keepdims=True)
            top = jnp.where(slot == c, best, top)
            key = jnp.where(key == best, 0.0, key)
        return pltpu.bitcast(top, I32) - 0x08000000

    def picked_tokens(top):
        return [(S - 1) - (top[c, 0] & (S - 1)) for c in range(CAP)]

    def gather(top):
        row = lax.broadcasted_iota(I32, (16, D), 0)
        slot = lax.broadcasted_iota(I32, (CAP, D), 0)
        xs = jnp.zeros((CAP, D), F32)
        for c, t in enumerate(picked_tokens(top)):
            near = xn_ref[span(t >> 4, 16), :].astype(F32)
            xs = jnp.where(slot == c, jnp.sum(jnp.where(row == (t & 15), near, 0.0), axis=0, keepdims=True), xs)
        return xs

    def panel_step(i, y):
        panel, part = 1 + i // parts1, i % parts1

        @pl.when(part == 0)
        def _():
            wq_copy(panel).wait()

        @pl.when(i == 0)
        def _():
            start(group_copies(0))

        @pl.when(i == 1)
        def _():
            wait(ffn_copies)

        hidden = pl.ds(pl.multiple_of(jnp.where(i == 0, wg_ref.shape[0] // FC - 1, i - 1) * FC, FC), FC)
        xs = xs_ref[...].astype(BF16)
        st = {}

        def ffn(n):
            k = n % (D // 128)
            cols = slice(k * 128, (k + 1) * 128)
            if n < 2 * (D // 128):
                ref = wg_ref if n < D // 128 else wu_ref
                t = lax.dot_general(xs[:, cols], ref[hidden, cols], NT, preferred_element_type=F32)
                st[n // (D // 128)] = t + st[n // (D // 128)] if k else t
            elif n < 3 * (D // 128):
                if k == 0:
                    st["h"] = (_bf(_silu(_bf(st[0]))) * _bf(st[1])).astype(BF16)
                st["y", k] = jnp.dot(st["h"], wd_ref[hidden, cols], preferred_element_type=F32)

        for b in range(P1 // R1):
            rows = span(part * (P1 // R1) + b, R1)
            xn = xn_ref[rows, :]
            if 'u' not in cfg['x']: upd_ref[rows, :] = jnp.zeros((R1, D), F32)
            for half in range(2):
                project_q(xn, panel, rows, half)
                n = 2 * b + half
                if n != 2 * (D // 128):
                    ffn(n - (n > 2 * (D // 128)))
        top = route()
        top_ref[...] = top
        xs_ref[...] = gather(top)
        return y + jnp.concatenate([st["y", k] for k in range(D // 128)], axis=1)

    y = lax.fori_loop(0, (panels - 1) * parts1, panel_step, jnp.zeros((CAP, D), F32))

    top = top_ref[...]
    rank = top >> 11
    r_sel = pltpu.bitcast(jnp.where(rank < 0x8000, ~rank, rank - 0x8000) << 16, F32)
    y = _bf(_bf(y) * _bf(jax.nn.sigmoid(r_sel[:, :1])))
    for c, t in enumerate(picked_tokens(top)):
        upd_ref[pl.ds(t, 1), :] = y[c:c + 1, :]

    def attend_step(i, carry):
        g, part = i // parts2, i % parts2

        @pl.when(part == 0)
        def _():
            wait(group_copies(g))

            @pl.when(g < groups - 1)
            def _():
                start(group_copies(g + 1))

        rows = lambda b: span(part * nb + b, R)
        per = QW // DH

        def store(b, a):
            acc_ref[rows(b), :] = a
            gate = _silu(xn_ref[rows(b), :].astype(F32) + upd_ref[rows(b), :])
            out_ref[rows(b), :] = (x_ref[rows(b), :].astype(F32) + a * gate).astype(out_ref.dtype)

        _attend(nb, ng,
                lambda b, h: q_ref[g * (ng // per) + h // per, rows(b), (h % per) * DH:(h % per + 1) * DH],
                lambda h, c: k_ref[g * ng + h, c * CK:(c + 1) * CK, :],
                lambda h, c: v_ref[g * ng + h, c * CK:(c + 1) * CK, :],
                lambda a, b: wo_ref[pl.ds(pl.multiple_of(g * (ng * DH), ng * DH) + a * DH, (b - a) * DH), :],
                lambda b: jnp.where(g > 0, acc_ref[rows(b), :], 0.0), store, cfg)

        @pl.when(g == groups - 1)
        def _():
            out_copy(part).start()

        return carry

    if cfg["skip"]:
        wait(group_copies(0))
        start([out_copy(p) for p in range(parts2)])
    else:
        lax.fori_loop(0, groups * parts2, attend_step, 0)
    wait([out_copy(p) for p in range(parts2)])


def make(R=64, CK=512, lead=6, epos=3, elast=7, eg=4, ng=16, nb=4, R0=64, P0=512, R1=128, P1=1024, FC=384, skip=False, x='u', pa=4, pc=3, flags=None):
    @jax.jit
    def fn(A_x, A_k_cache, A_v_cache, A_wq, A_wo, B_x, B_w_r, B_w_gate, B_w_up, B_w_down):
        B, S, D = A_x.shape
        Sk = A_k_cache.shape[2]
        cfg = dict(R=R, CK=CK, lead=lead, epos=epos, elast=elast, eg=eg, ng=ng, nb=nb, R0=R0, P0=P0, R1=R1, P1=P1,
                   FC=FC, Sk=Sk, skip=skip, x=x, pa=pa, pc=pc)
        panels = H * DH // QW
        Fp = (panels - 1) * (S // P1) * FC
        hbm = pl.BlockSpec(memory_space=pltpu.HBM)
        vmem, dma = pltpu.VMEM, pltpu.SemaphoreType.DMA
        return pl.pallas_call(
            functools.partial(_kernel, cfg=cfg),
            in_specs=[hbm] * 9,
            out_specs=hbm,
            out_shape=jax.ShapeDtypeStruct((B, S, D), A_x.dtype),
            scratch_shapes=[
                vmem((S, D), BF16), vmem((S, D), BF16), vmem((S, D), F32), vmem((S, D), F32), vmem((S, D), A_x.dtype),
                vmem((panels, S, QW), BF16), vmem((H, Sk, DH), BF16), vmem((H, Sk, DH), BF16),
                vmem((panels, D, QW), BF16), vmem((H * DH, D), BF16),
                vmem((Fp, D), BF16), vmem((Fp, D), BF16), vmem((Fp, D), BF16),
                vmem((CAP, D), F32), vmem((R0, D), BF16), vmem((S // P0, 8, 128), F32), vmem((CAP, 128), I32),
                vmem((D,), BF16),
                dma((S // P0,)), dma((panels,)), dma((4,)), dma((H // ng, 3)), dma((S // (nb * R),)),
            ],
            compiler_params=pltpu.CompilerParams(
                vmem_limit_bytes=112 * 1024 * 1024, internal_scratch_in_bytes=64 * 1024, flags=flags),
        )(A_x, A_k_cache, A_v_cache, A_wq, A_wo, B_w_r, B_w_gate.T, B_w_up.T, B_w_down)
    return fn


pallas_recurrent_scan__mha_block_cached__moe_arch_mod__prompt_kernel = make()
```

```python
import functools
import math

import jax
import jax.numpy as jnp
from jax import lax
import jax.experimental.pallas as pl
import jax.experimental.pallas.tpu as pltpu

F32 = jnp.float32
BF16 = jnp.bfloat16
I32 = jnp.int32

H, DH = 32, 128
CAP = 8
EPS = 1e-5
NT = (((1,), (1,)), ((), ()))
QW = 8 * DH


def _divmod(i, n):
    assert n & (n - 1) == 0
    return i >> (n.bit_length() - 1), i & (n - 1)


def _bf(x):
    return x.astype(BF16).astype(F32)


def _silu(x):
    h = 0.5 * x
    return h + h * jnp.tanh(h)


def _after(x, other, zero):
    bits = pltpu.bitcast(x, I32) | (pltpu.bitcast(other, I32) & jnp.full(x.shape, zero, I32))
    return pltpu.bitcast(bits, F32)


def _layernorm(x, pace=None):
    d = x.shape[-1]
    x = x.astype(F32)
    if pace is not None:
        x = jnp.concatenate([_after(x[:, :128], *pace), x[:, 128:]], axis=1)
    mu = jnp.sum(x, axis=-1, keepdims=True) * (1.0 / d)
    xc = x - mu
    var = jnp.sum(xc * xc, axis=-1, keepdims=True) * (1.0 / d)
    den = _bf(jnp.sqrt(_bf(_bf(var) + _bf(jnp.full_like(var, EPS)))))
    inv = pl.reciprocal(den, approx=True)
    inv = jnp.where(den == jnp.inf, 0.0, inv * (2.0 - den * inv))
    return (_bf(x - _bf(mu)) * inv).astype(BF16)


class _Attention:
    def __init__(self, cfg, query, keys, vals):
        self.R, self.CK, self.nck = cfg["R"], cfg["CK"], cfg["Sk"] // cfg["CK"]
        self.query, self.keys, self.vals = query, keys, vals
        self.q, self.s, self.m, self.l, self.o = {}, {}, {}, {}, {}

    def scores(self, j):
        u, c = divmod(j, self.nck)
        if u not in self.q:
            self.q[u] = self.query(u)
        s = self.s[j] = lax.dot_general(self.q[u], self.keys(u, c), NT, preferred_element_type=F32)
        m = jnp.maximum(s[:, :128], self.m[u]) if c else s[:, :128]
        for t in range(1, self.CK // 128):
            m = jnp.maximum(m, s[:, t * 128:(t + 1) * 128])
        if c == self.nck - 1:
            m = jnp.broadcast_to(jnp.max(m, axis=-1, keepdims=True), m.shape)
        self.m[u] = m

    def values(self, j):
        u, c = divmod(j, self.nck)
        p = jnp.exp2(self.s[j] - jnp.concatenate([self.m[u]] * (self.CK // 128), axis=1))
        l = p[:, :128] + self.l[u] if c else p[:, :128]
        for t in range(1, self.CK // 128):
            l = l + p[:, t * 128:(t + 1) * 128]
        self.l[u] = l
        p = jnp.concatenate([p[:, :-128], jnp.minimum(p[:, -128:], l)], axis=1)
        o = jnp.dot(p.astype(BF16), self.vals(u, c), preferred_element_type=F32)
        self.o[u] = o + self.o[u] if c else o


def _merge_heads(pairs):
    heads = []
    for o, l in pairs:
        l = jnp.sum(l, axis=-1, keepdims=True)
        r = pl.reciprocal(l, approx=True)
        heads.append(o * (r * (2.0 - l * r)))
    return jnp.concatenate(heads, axis=1).astype(BF16)


def _kernel(x_hbm, k_hbm, v_hbm, wq_hbm, wo_hbm, wr_hbm, wg_hbm, wu_hbm, wd_hbm, out_hbm,
            x_ref, xn_ref, upd_ref, acc_ref, out_ref, q_ref, k_ref, v_ref, wq_ref, wo_ref,
            wg_ref, wu_ref, wd_ref, s_ref, m_ref, tail_ref, part_ref, xs_ref, head_ref, score_ref, top_ref, wr_ref,
            x_sem, q_sem, w_sem, p_sem, o_sem, *, cfg):
    S, D = x_ref.shape
    F = wg_hbm.shape[0]
    R, CK, ng, nb = cfg["R"], cfg["CK"], cfg["ng"], cfg["nb"]
    R0, P0, R1, P1, FC = cfg["R0"], cfg["P0"], cfg["R1"], cfg["P1"], cfg["FC"]
    panels, groups = H * DH // QW, H // ng
    parts0, parts1, parts2 = S // P0, S // P1, S // (nb * R)
    qscale = (DH ** -0.5) * math.log2(math.e)

    def span(i, n):
        return pl.ds(i * n if isinstance(i, int) else pl.multiple_of(i * n, n), n)

    def x_copy(i):
        rows = slice(i * P0 + R0, min((i + 1) * P0 + R0, S)) if i < parts0 else slice(0, R0)
        return pltpu.make_async_copy(x_hbm.at[0, rows], x_ref.at[rows], x_sem.at[i])

    def wq_copy(i):
        return pltpu.make_async_copy(wq_hbm.at[:, span(i, QW)], wq_ref.at[i], q_sem.at[i])

    def group_copies(g):
        return [pltpu.make_async_copy(k_hbm.at[0, span(g, ng)], k_ref.at[span(g, ng)], p_sem.at[g, 0]),
                pltpu.make_async_copy(v_hbm.at[0, span(g, ng)], v_ref.at[span(g, ng)], p_sem.at[g, 1]),
                pltpu.make_async_copy(wo_hbm.at[span(g, ng * DH)], wo_ref.at[span(g, ng * DH)], p_sem.at[g, 2])]

    def out_copy(i):
        rows = span(i, nb * R)
        if isinstance(i, int) and i >= parts2 - 1:
            rows = pl.ds(S - nb * R, (nb - 1) * R) if i < parts2 else pl.ds(S - R, R)
        return pltpu.make_async_copy(out_ref.at[rows], out_hbm.at[0, rows], o_sem.at[i])

    wr_copy = pltpu.make_async_copy(wr_hbm, wr_ref, w_sem.at[0])
    ffn_copies = [pltpu.make_async_copy(src, dst.at[:F], w_sem.at[i + 1])
                  for i, (src, dst) in enumerate([(wg_hbm, wg_ref), (wu_hbm, wu_ref), (wd_hbm, wd_ref)])]

    def start(copies):
        for c in copies:
            c.start()

    def wait(copies):
        for c in copies:
            c.wait()

    def project_q(xn, panel, rows, half):
        cols = slice(half * QW // 2, (half + 1) * QW // 2)
        q = jnp.dot(xn, wq_ref[panel, :, cols], preferred_element_type=F32)
        q_ref[panel, rows, cols] = (q * qscale).astype(BF16)
        return q

    start([x_copy(parts0), wr_copy, wq_copy(0), x_copy(0)])
    for ref in (wg_ref, wu_ref, wd_ref):
        ref[F:, :] = jnp.zeros((ref.shape[0] - F, D), BF16)
    xs_ref[...] = jnp.zeros_like(xs_ref)
    wait([x_copy(parts0)])
    head_ref[...] = _layernorm(x_ref[:R0, :])
    wait([wr_copy, wq_copy(0), x_copy(0)])
    start([x_copy(i) for i in range(1, parts0)] + [wq_copy(1)])

    lane = lax.broadcasted_iota(I32, (8, 128), 1)
    per_part = P0 // 8

    def norm_step(i, carry):
        for j in range(1, parts0):
            pl.when(i == j)(x_copy(j).wait)

        @pl.when(i == 1)
        def _():
            start(ffn_copies + [wq_copy(j) for j in range(2, panels)])

        wr = wr_ref[...].astype(F32).reshape(1, D)
        score = jnp.zeros((8, 128), F32)
        late, done = [], []
        pace = lambda b: (done[2 * b - cfg['pa']][:, cfg['pc'] * 128:(cfg['pc'] + 1) * 128], i >> 8) if 2 * b >= cfg['pa'] else None
        for b in range(P0 // R0):
            rows = span(i * (P0 // R0) + b, R0)
            xn = head_ref[...] if b == 0 else _layernorm(x_ref[rows, :], pace(b))
            if "n" in cfg["x"]: late.append((rows, xn))
            else: xn_ref[rows, :] = xn
            r = jnp.sum(xn.astype(F32) * wr, axis=-1, keepdims=True) if 'r' not in cfg['x'] else xn.astype(F32)[:, :128]
            for j in range(R0 // 8):
                score = jnp.where(lane % per_part == b * (R0 // 8) + j, r[j * 8:(j + 1) * 8], score)
            if "u" in cfg["x"]: upd_ref[rows, :] = jnp.zeros((R0, D), F32)
            done.append(project_q(xn, 0, rows, 0))
            done.append(project_q(xn, 0, rows, 1))
        score_ref[i] = score
        for rows, xn in late: xn_ref[rows, :] = xn
        ahead = jnp.minimum(i + 1, parts0 - 1) * (P0 // R0)
        head_ref[...] = _layernorm(x_ref[span(ahead, R0), :], pace(P0 // R0))
        return carry

    lax.fori_loop(0, parts0, norm_step, 0)

    def route():
        tiles = []
        for t in range(S // 1024):
            ps = range(t * (128 // per_part), (t + 1) * (128 // per_part))
            tile = score_ref[ps[0]]
            for j, p in enumerate(ps[1:]):
                tile = jnp.where(lane // per_part == j + 1, score_ref[p], tile)
            tiles.append(tile)
        r = _bf(jnp.concatenate(tiles, axis=1))
        r = jnp.where(r == 0.0, 0.0, r)
        bits = pltpu.bitcast(r, I32) >> 16
        rank = jnp.where(r != r, 0, jnp.where(bits < 0, ~bits, bits + 0x8000))
        token = lax.broadcasted_iota(I32, r.shape, 1) * 8 + lax.broadcasted_iota(I32, r.shape, 0)
        key = pltpu.bitcast(((rank << 11) | (S - 1 - token)) + 0x08000000, F32)
        slot = lax.broadcasted_iota(I32, (CAP, 128), 0)
        top = jnp.zeros((CAP, 128), F32)
        for c in range(CAP):
            best = jnp.max(jnp.max(key, axis=0, keepdims=True), axis=1, keepdims=True)
            top = jnp.where(slot == c, best, top)
            key = jnp.where(key == best, 0.0, key)
        return pltpu.bitcast(top, I32) - 0x08000000

    def picked_tokens(top):
        return [(S - 1) - (top[c, 0] & (S - 1)) for c in range(CAP)]

    def gather(top):
        row = lax.broadcasted_iota(I32, (16, D), 0)
        slot = lax.broadcasted_iota(I32, (CAP, D), 0)
        xs = jnp.zeros((CAP, D), F32)
        for c, t in enumerate(picked_tokens(top)):
            near = xn_ref[span(t >> 4, 16), :].astype(F32)
            xs = jnp.where(slot == c, jnp.sum(jnp.where(row == (t & 15), near, 0.0), axis=0, keepdims=True), xs)
        return xs

    def panel_step(i, y):
        panel, part = _divmod(i + parts1, parts1)

        @pl.when(part == 0)
        def _():
            wq_copy(panel).wait()

        @pl.when(i == 0)
        def _():
            start(group_copies(0))

        @pl.when(i == 1)
        def _():
            wait(ffn_copies)

        hidden = pl.ds(pl.multiple_of(jnp.where(i == 0, wg_ref.shape[0] // FC - 1, i - 1) * FC, FC), FC)
        xs = xs_ref[...].astype(BF16)
        st = {}

        def ffn(n):
            k = n % (D // 128)
            cols = slice(k * 128, (k + 1) * 128)
            if n < 2 * (D // 128):
                ref = wg_ref if n < D // 128 else wu_ref
                t = lax.dot_general(xs[:, cols], ref[hidden, cols], NT, preferred_element_type=F32)
                st[n // (D // 128)] = t + st[n // (D // 128)] if k else t
            elif n < 3 * (D // 128):
                if k == 0:
                    st["h"] = (_bf(_silu(_bf(st[0]))) * _bf(st[1])).astype(BF16)
                st["y", k] = jnp.dot(st["h"], wd_ref[hidden, cols], preferred_element_type=F32)

        for b in range(P1 // R1):
            rows = span(part * (P1 // R1) + b, R1)
            xn = xn_ref[rows, :]
            if 'u' not in cfg['x']: upd_ref[rows, :] = jnp.zeros((R1, D), F32)
            for half in range(2):
                project_q(xn, panel, rows, half)
                n = 2 * b + half
                if n != 2 * (D // 128):
                    ffn(n - (n > 2 * (D // 128)))
        top = route()
        top_ref[...] = top
        xs_ref[...] = gather(top)
        return y + jnp.concatenate([st["y", k] for k in range(D // 128)], axis=1)

    y = lax.fori_loop(0, (panels - 1) * parts1, panel_step, jnp.zeros((CAP, D), F32))

    nck, lead, eg = cfg["Sk"] // CK, cfg["lead"], cfg["eg"]
    units, steps, per = nb * ng, groups * parts2, QW // DH

    def attention(i):
        after = min(i + 1, steps - 1) if isinstance(i, int) else jnp.minimum(i + 1, steps - 1)

        def place(u):
            step = i if u < units else after
            b, h = divmod(u % units, ng)
            g, part = _divmod(step, parts2)
            return g, span(part * nb + b, R), h

        def query(u):
            g, rows, h = place(u)
            return q_ref[g * (ng // per) + h // per, rows, (h % per) * DH:(h % per + 1) * DH]

        def cache(ref, u, c):
            g, _, h = place(u)
            return ref[g * ng + h, c * CK:(c + 1) * CK, :]

        return _Attention(cfg, query, functools.partial(cache, k_ref), functools.partial(cache, v_ref))

    def hand_over(att, first):
        for j in range(lead):
            s_ref[j] = att.s[first + j]
        for u in range(pl.cdiv(lead, nck)):
            m_ref[u] = att.m[first // nck + u]

    def project(o, g, h0, a):
        w = wo_ref[pl.ds(pl.multiple_of(g * (ng * DH), ng * DH) + h0 * DH, o.shape[1]), :]
        return jnp.dot(o, w, preferred_element_type=F32) + a

    def finish(rows, a):
        acc_ref[rows, :] = a
        gate = _silu(xn_ref[rows, :].astype(F32) + upd_ref[rows, :])
        out_ref[rows, :] = (x_ref[rows, :].astype(F32) + a * gate).astype(out_ref.dtype)

    def finish_previous(step):
        g, part = _divmod(step, parts2)
        finish(span(part * nb + nb - 1, R), project(_merge_heads([(tail_ref[0, h], tail_ref[1, h]) for h in range(eg)]),
                                                g, ng - eg, part_ref[...]))

    wait(group_copies(0))
    start([c for g in range(1, groups) for c in group_copies(g)])
    att = attention(0)
    for j in range(lead):
        att.scores(j)
    hand_over(att, 0)
    tail_ref[...] = jnp.ones_like(tail_ref)
    part_ref[...] = jnp.zeros_like(part_ref)
    top = top_ref[...]
    rank = top >> 11
    r_sel = pltpu.bitcast(jnp.where(rank < 0x8000, ~rank, rank - 0x8000) << 16, F32)
    y = _bf(_bf(y) * _bf(jax.nn.sigmoid(r_sel[:, :1])))
    for c, t in enumerate(picked_tokens(top)):
        upd_ref[pl.ds(t, 1), :] = y[c:c + 1, :]

    def attend_step(i, carry):
        g, part = _divmod(i, parts2)
        for nxt in range(1, groups):
            pl.when(i == nxt * parts2 - 1)(functools.partial(wait, group_copies(nxt)))

        att = attention(i)
        for j in range(lead):
            att.s[j] = s_ref[j]
        for u in range(pl.cdiv(lead, nck)):
            att.m[u] = m_ref[u]
        acc = {}

        def project_heads(b, h0):
            rows = span(part * nb + b, R)
            a = acc[b] if h0 else jnp.where(g > 0, acc_ref[rows, :], 0.0)
            acc[b] = project(_merge_heads([(att.o[u], att.l[u]) for u in range(b * ng + h0, b * ng + h0 + eg)]), g, h0, a)
            if h0 + eg == ng:
                finish(rows, acc[b])

        prog = [((cfg["epos"], 4), finish_previous, (jnp.maximum(i - 1, 0),))]
        for j in range(units * nck):
            prog.append(((j, cfg["bpos"]), att.scores, (j + lead,)))
            prog.append(((j, 3), att.values, (j,)))
        for u in range(eg, units, eg):
            prog.append(((u * nck + cfg["epos"], 4), project_heads, divmod(u - eg, ng)))
        for _, fn, args in sorted(prog, key=lambda e: e[0]):
            fn(*args)
        hand_over(att, units * nck)
        for h in range(eg):
            tail_ref[0, h] = att.o[units - eg + h]
            tail_ref[1, h] = att.l[units - eg + h]
        part_ref[...] = acc[nb - 1]

        @pl.when(i > steps - parts2)
        def _():
            out_copy(part - 1).start()

        return carry

    lax.fori_loop(0, steps, attend_step, 0)
    out_copy(parts2 - 1).start()
    finish_previous(steps - 1)
    out_copy(parts2).start()
    wait([out_copy(p) for p in range(parts2 + 1)])


def make(R=64, CK=512, lead=7, epos=3, bpos=3.5, eg=4, ng=16, nb=4, R0=64, P0=512, R1=128, P1=1024, FC=384, skip=False, x='u', pa=4, pc=3, flags=None):
    @jax.jit
    def fn(A_x, A_k_cache, A_v_cache, A_wq, A_wo, B_x, B_w_r, B_w_gate, B_w_up, B_w_down):
        B, S, D = A_x.shape
        Sk = A_k_cache.shape[2]
        cfg = dict(R=R, CK=CK, lead=lead, epos=epos, bpos=bpos, eg=eg, ng=ng, nb=nb, R0=R0, P0=P0, R1=R1, P1=P1,
                   FC=FC, Sk=Sk, skip=skip, x=x, pa=pa, pc=pc)
        panels = H * DH // QW
        Fp = (panels - 1) * (S // P1) * FC
        hbm = pl.BlockSpec(memory_space=pltpu.HBM)
        vmem, dma = pltpu.VMEM, pltpu.SemaphoreType.DMA
        return pl.pallas_call(
            functools.partial(_kernel, cfg=cfg),
            in_specs=[hbm] * 9,
            out_specs=hbm,
            out_shape=jax.ShapeDtypeStruct((B, S, D), A_x.dtype),
            scratch_shapes=[
                vmem((S, D), BF16), vmem((S, D), BF16), vmem((S, D), F32), vmem((S, D), F32), vmem((S, D), A_x.dtype),
                vmem((panels, S, QW), BF16), vmem((H, Sk, DH), BF16), vmem((H, Sk, DH), BF16),
                vmem((panels, D, QW), BF16), vmem((H * DH, D), BF16),
                vmem((Fp, D), BF16), vmem((Fp, D), BF16), vmem((Fp, D), BF16),
                vmem((lead, R, CK), F32), vmem((pl.cdiv(lead * CK, Sk), R, 128), F32), vmem((2, eg, R, DH), F32), vmem((R, D), F32),
                vmem((CAP, D), F32), vmem((R0, D), BF16), vmem((S // P0, 8, 128), F32), vmem((CAP, 128), I32),
                vmem((D,), BF16),
                dma((S // P0 + 1,)), dma((panels,)), dma((4,)), dma((H // ng, 3)), dma((S // (nb * R) + 1,)),
            ],
            compiler_params=pltpu.CompilerParams(
                vmem_limit_bytes=112 * 1024 * 1024, internal_scratch_in_bytes=64 * 1024, flags=flags),
        )(A_x, A_k_cache, A_v_cache, A_wq, A_wo, B_w_r, B_w_gate.T, B_w_up.T, B_w_down)
    return fn


pallas_recurrent_scan__mha_block_cached__moe_arch_mod__prompt_kernel = make()
```

```python
import functools
import math

import jax
import jax.numpy as jnp
from jax import lax
import jax.experimental.pallas as pl
import jax.experimental.pallas.tpu as pltpu

F32 = jnp.float32
BF16 = jnp.bfloat16
I32 = jnp.int32

H, DH = 32, 128
CAP = 8
EPS = 1e-5
NT = (((1,), (1,)), ((), ()))
QW = 8 * DH


def _divmod(i, n):
    assert n & (n - 1) == 0
    return i >> (n.bit_length() - 1), i & (n - 1)


def _bf(x):
    return x.astype(BF16).astype(F32)


def _silu(x):
    h = 0.5 * x
    return h + h * jnp.tanh(h)


def _after(x, other):
    return jnp.where(other > jnp.inf, other, x)


def _layernorm(x, pace=None):
    d = x.shape[-1]
    x = x.astype(F32)
    if pace is not None:
        x = jnp.concatenate([_after(x[:, :128], pace), x[:, 128:]], axis=1)
    mu = jnp.sum(x, axis=-1, keepdims=True) * (1.0 / d)
    xc = x - mu
    var = jnp.sum(xc * xc, axis=-1, keepdims=True) * (1.0 / d)
    den = _bf(jnp.sqrt(_bf(_bf(var) + _bf(jnp.full_like(var, EPS)))))
    inv = pl.reciprocal(den, approx=True)
    inv = jnp.where(den == jnp.inf, 0.0, inv * (2.0 - den * inv))
    return (_bf(x - _bf(mu)) * inv).astype(BF16)


class _Attention:
    def __init__(self, cfg, query, keys, vals):
        self.R, self.CK, self.nck = cfg["R"], cfg["CK"], cfg["Sk"] // cfg["CK"]
        self.query, self.keys, self.vals = query, keys, vals
        self.q, self.s, self.m, self.l, self.o = {}, {}, {}, {}, {}

    def scores(self, j):
        u, c = divmod(j, self.nck)
        if u not in self.q:
            self.q[u] = self.query(u)
        s = self.s[j] = lax.dot_general(self.q[u], self.keys(u, c), NT, preferred_element_type=F32)
        m = jnp.maximum(s[:, :128], self.m[u]) if c else s[:, :128]
        for t in range(1, self.CK // 128):
            m = jnp.maximum(m, s[:, t * 128:(t + 1) * 128])
        if c == self.nck - 1:
            m = jnp.broadcast_to(jnp.max(m, axis=-1, keepdims=True), m.shape)
        self.m[u] = m

    def values(self, j):
        u, c = divmod(j, self.nck)
        p = jnp.exp2(self.s[j] - jnp.concatenate([self.m[u]] * (self.CK // 128), axis=1))
        l = p[:, :128] + self.l[u] if c else p[:, :128]
        for t in range(1, self.CK // 128):
            l = l + p[:, t * 128:(t + 1) * 128]
        self.l[u] = l
        p = jnp.concatenate([p[:, :-128], jnp.minimum(p[:, -128:], l)], axis=1)
        o = jnp.dot(p.astype(BF16), self.vals(u, c), preferred_element_type=F32)
        self.o[u] = o + self.o[u] if c else o


def _merge_heads(pairs):
    heads = []
    for o, l in pairs:
        l = jnp.sum(l, axis=-1, keepdims=True)
        r = pl.reciprocal(l, approx=True)
        heads.append(o * (r * (2.0 - l * r)))
    return jnp.concatenate(heads, axis=1).astype(BF16)


def _kernel(x_hbm, k_hbm, v_hbm, wq_hbm, wo_hbm, wr_hbm, wg_hbm, wu_hbm, wd_hbm, out_hbm,
            x_ref, xn_ref, upd_ref, acc_ref, out_ref, q_ref, k_ref, v_ref, wq_ref, wo_ref,
            wg_ref, wu_ref, wd_ref, s_ref, m_ref, tail_ref, part_ref, xs_ref, head_ref, score_ref, top_ref, wr_ref,
            x_sem, f_sem, q_sem, w_sem, p_sem, o_sem, *, cfg):
    S, D = x_ref.shape
    F = wg_hbm.shape[0]
    R, CK, ng, nb = cfg["R"], cfg["CK"], cfg["ng"], cfg["nb"]
    R0, P0, R1, P1, FC = cfg["R0"], cfg["P0"], cfg["R1"], cfg["P1"], cfg["FC"]
    panels, groups = H * DH // QW, H // ng
    parts0, parts1, parts2 = S // P0, S // P1, S // (nb * R)
    qscale = (DH ** -0.5) * math.log2(math.e)

    def span(i, n):
        return pl.ds(i * n if isinstance(i, int) else pl.multiple_of(i * n, n), n)

    def wq_copy(i):
        return pltpu.make_async_copy(wq_hbm.at[:, span(i, QW)], wq_ref.at[i], q_sem.at[i])

    def group_copies(g):
        return [pltpu.make_async_copy(k_hbm.at[0, span(g, ng)], k_ref.at[span(g, ng)], p_sem.at[g, 0]),
                pltpu.make_async_copy(v_hbm.at[0, span(g, ng)], v_ref.at[span(g, ng)], p_sem.at[g, 1]),
                pltpu.make_async_copy(wo_hbm.at[span(g, ng * DH)], wo_ref.at[span(g, ng * DH)], p_sem.at[g, 2])]

    def out_copy(i):
        rows = span(i, nb * R)
        if isinstance(i, int) and i >= parts2 - 1:
            rows = pl.ds(S - nb * R, (nb - 1) * R) if i < parts2 else pl.ds(S - R, R)
        return pltpu.make_async_copy(out_ref.at[rows], out_hbm.at[0, rows], o_sem.at[i])

    wr_copy = pltpu.make_async_copy(wr_hbm, wr_ref, w_sem.at[0])
    ffn_copies = [pltpu.make_async_copy(src, dst.at[:F], w_sem.at[i + 1])
                  for i, (src, dst) in enumerate([(wg_hbm, wg_ref), (wu_hbm, wu_ref), (wd_hbm, wd_ref)])]

    def start(copies):
        for c in copies:
            c.start()

    def wait(copies):
        for c in copies:
            c.wait()

    def project_q(xn, panel, rows, half):
        cols = slice(half * QW // 2, (half + 1) * QW // 2)
        q = jnp.dot(xn, wq_ref[panel, :, cols], preferred_element_type=F32)
        q_ref[panel, rows, cols] = (q * qscale).astype(BF16)
        return q

    lane = lax.broadcasted_iota(I32, (8, 128), 1)
    per_part = P0 // 8
    nb0, early = P0 // R0, cfg["early"]

    def keep(i, normed):
        wr = wr_ref[...].astype(F32).reshape(1, D)
        score = jnp.zeros((8, 128), F32)
        for b, xn in enumerate(normed):
            xn_ref[span(i * nb0 + b, R0), :] = xn
            upd_ref[span(i * nb0 + b, R0), :] = jnp.zeros((R0, D), F32)
            r = jnp.sum(xn.astype(F32) * wr, axis=-1, keepdims=True)
            for j in range(R0 // 8):
                score = jnp.where(lane % per_part == b * (R0 // 8) + j, r[j * 8:(j + 1) * 8], score)
        score_ref[i] = score

    edges = [0, early * R0] + [i * P0 + R0 for i in range(1, parts0)] + [S]
    x_copies = [pltpu.make_async_copy(x_hbm.at[0, a:b], x_ref.at[a:b], x_sem.at[i])
                for i, (a, b) in enumerate(zip(edges, edges[1:]))]
    wq_first = [pltpu.make_async_copy(wq_hbm.at[:, span(i, QW // 2)], wq_ref.at[0, :, span(i, QW // 2)], f_sem.at[i])
                for i in range(2)]

    start([x_copies[0], wq_first[0], x_copies[1], wq_first[1]])
    for ref in (wg_ref, wu_ref, wd_ref):
        ref[F:, :] = jnp.zeros((ref.shape[0] - F, D), BF16)
    xs_ref[...] = jnp.zeros_like(xs_ref)
    wait([x_copies[0]])
    normed = [_layernorm(x_ref[span(b, R0), :]) for b in range(early)]
    wait([wq_first[0]])
    done = []
    for b in range(nb0):
        if b == early - 2:
            wait([x_copies[1]])
            start([wr_copy, x_copies[2]])
        if b >= early:
            normed.append(_layernorm(x_ref[span(b, R0), :]))
        done.append(project_q(normed[b], 0, span(b, R0), 0))
    wait([wq_first[1], wr_copy])
    start(x_copies[3:])
    for b in range(nb0):
        project_q(normed[b], 0, span(b, R0), 1)
    keep(0, normed)
    head_ref[...] = _layernorm(x_ref[span(nb0, R0), :])

    def norm_step(i, carry):
        for j in range(1, parts0):
            pl.when(i == j)(x_copies[j + 1].wait)
        pl.when(i == 1)(functools.partial(start, [wq_copy(1)] + ffn_copies))
        pl.when(i == parts0 - 1)(functools.partial(start, [wq_copy(j) for j in range(2, panels)]))
        normed, done = [head_ref[...]], []

        def pace(b):
            n, per = cfg["pn"], QW // 256
            first = 2 * per * b - cfg["pa"]
            if first < 0:
                return None
            tiles = [divmod(first + j * cfg["pc"], per) for j in range(R0 // n)]
            return jnp.concatenate([done[d][j * n:(j + 1) * n, t * 128:(t + 1) * 128] for j, (d, t) in enumerate(tiles)], axis=0)

        for b in range(nb0):
            rows = span(i * nb0 + b, R0)
            if b:
                normed.append(_layernorm(x_ref[rows, :], pace(b)))
            done.append(project_q(normed[b], 0, rows, 0))
            done.append(project_q(normed[b], 0, rows, 1))
        keep(i, normed)
        head_ref[...] = _layernorm(x_ref[span(jnp.minimum(i + 1, parts0 - 1) * nb0, R0), :], pace(nb0))
        return carry

    lax.fori_loop(1, parts0, norm_step, 0)

    def route():
        tiles = []
        for t in range(S // 1024):
            ps = range(t * (128 // per_part), (t + 1) * (128 // per_part))
            tile = score_ref[ps[0]]
            for j, p in enumerate(ps[1:]):
                tile = jnp.where(lane // per_part == j + 1, score_ref[p], tile)
            tiles.append(tile)
        r = _bf(jnp.concatenate(tiles, axis=1))
        r = jnp.where(r == 0.0, 0.0, r)
        bits = pltpu.bitcast(r, I32) >> 16
        rank = jnp.where(r != r, 0, jnp.where(bits < 0, ~bits, bits + 0x8000))
        token = lax.broadcasted_iota(I32, r.shape, 1) * 8 + lax.broadcasted_iota(I32, r.shape, 0)
        key = pltpu.bitcast(((rank << 11) | (S - 1 - token)) + 0x08000000, F32)
        slot = lax.broadcasted_iota(I32, (CAP, 128), 0)
        top = jnp.zeros((CAP, 128), F32)
        for c in range(CAP):
            best = jnp.max(jnp.max(key, axis=0, keepdims=True), axis=1, keepdims=True)
            top = jnp.where(slot == c, best, top)
            key = jnp.where(key == best, 0.0, key)
        return pltpu.bitcast(top, I32) - 0x08000000

    def picked_tokens(top):
        return [(S - 1) - (top[c, 0] & (S - 1)) for c in range(CAP)]

    def gather(top):
        row = lax.broadcasted_iota(I32, (16, D), 0)
        slot = lax.broadcasted_iota(I32, (CAP, D), 0)
        xs = jnp.zeros((CAP, D), F32)
        for c, t in enumerate(picked_tokens(top)):
            near = xn_ref[span(t >> 4, 16), :].astype(F32)
            xs = jnp.where(slot == c, jnp.sum(jnp.where(row == (t & 15), near, 0.0), axis=0, keepdims=True), xs)
        return xs

    def panel_step(i, y):
        panel, part = _divmod(i + parts1, parts1)

        @pl.when(part == 0)
        def _():
            wq_copy(panel).wait()

        @pl.when(i == 0)
        def _():
            start(group_copies(0))

        @pl.when(i == 1)
        def _():
            wait(ffn_copies)

        hidden = pl.ds(pl.multiple_of(jnp.where(i == 0, wg_ref.shape[0] // FC - 1, i - 1) * FC, FC), FC)
        xs = xs_ref[...].astype(BF16)
        st = {}

        def ffn(n):
            k = n % (D // 128)
            cols = slice(k * 128, (k + 1) * 128)
            if n < 2 * (D // 128):
                ref = wg_ref if n < D // 128 else wu_ref
                t = lax.dot_general(xs[:, cols], ref[hidden, cols], NT, preferred_element_type=F32)
                st[n // (D // 128)] = t + st[n // (D // 128)] if k else t
            elif n < 3 * (D // 128):
                if k == 0:
                    st["h"] = (_bf(_silu(_bf(st[0]))) * _bf(st[1])).astype(BF16)
                st["y", k] = jnp.dot(st["h"], wd_ref[hidden, cols], preferred_element_type=F32)

        for b in range(P1 // R1):
            rows = span(part * (P1 // R1) + b, R1)
            xn = xn_ref[rows, :]
            for half in range(2):
                project_q(xn, panel, rows, half)
                n = 2 * b + half
                if n != 2 * (D // 128):
                    ffn(n - (n > 2 * (D // 128)))
        top = route()
        top_ref[...] = top
        xs_ref[...] = gather(top)
        return y + jnp.concatenate([st["y", k] for k in range(D // 128)], axis=1)

    y = lax.fori_loop(0, (panels - 1) * parts1, panel_step, jnp.zeros((CAP, D), F32))

    nck, lead, eg = cfg["Sk"] // CK, cfg["lead"], cfg["eg"]
    units, steps, per = nb * ng, groups * parts2, QW // DH

    def attention(i):
        after = min(i + 1, steps - 1) if isinstance(i, int) else jnp.minimum(i + 1, steps - 1)

        def place(u):
            step = i if u < units else after
            b, h = divmod(u % units, ng)
            g, part = _divmod(step, parts2)
            return g, span(part * nb + b, R), h

        def query(u):
            g, rows, h = place(u)
            return q_ref[g * (ng // per) + h // per, rows, (h % per) * DH:(h % per + 1) * DH]

        def cache(ref, u, c):
            g, _, h = place(u)
            return ref[g * ng + h, c * CK:(c + 1) * CK, :]

        return _Attention(cfg, query, functools.partial(cache, k_ref), functools.partial(cache, v_ref))

    def hand_over(att, first):
        for j in range(lead):
            s_ref[j] = att.s[first + j]
        for u in range(pl.cdiv(lead, nck)):
            m_ref[u] = att.m[first // nck + u]

    def project(o, g, h0, a):
        w = wo_ref[pl.ds(pl.multiple_of(g * (ng * DH), ng * DH) + h0 * DH, o.shape[1]), :]
        return jnp.dot(o, w, preferred_element_type=F32) + a

    def finish(rows, a):
        acc_ref[rows, :] = a
        gate = _silu(xn_ref[rows, :].astype(F32) + upd_ref[rows, :])
        out_ref[rows, :] = (x_ref[rows, :].astype(F32) + a * gate).astype(out_ref.dtype)

    def finish_previous(step):
        g, part = _divmod(step, parts2)
        finish(span(part * nb + nb - 1, R), project(_merge_heads([(tail_ref[0, h], tail_ref[1, h]) for h in range(eg)]),
                                                g, ng - eg, part_ref[...]))

    wait(group_copies(0))
    start([c for g in range(1, groups) for c in group_copies(g)])
    att = attention(0)
    for j in range(lead):
        att.scores(j)
    hand_over(att, 0)
    tail_ref[...] = jnp.ones_like(tail_ref)
    part_ref[...] = jnp.zeros_like(part_ref)
    top = top_ref[...]
    rank = top >> 11
    r_sel = pltpu.bitcast(jnp.where(rank < 0x8000, ~rank, rank - 0x8000) << 16, F32)
    y = _bf(_bf(y) * _bf(jax.nn.sigmoid(r_sel[:, :1])))
    for c, t in enumerate(picked_tokens(top)):
        upd_ref[pl.ds(t, 1), :] = y[c:c + 1, :]

    def attend_step(i, carry):
        g, part = _divmod(i, parts2)
        for nxt in range(1, groups):
            pl.when(i == nxt * parts2 - 1)(functools.partial(wait, group_copies(nxt)))

        att = attention(i)
        for j in range(lead):
            att.s[j] = s_ref[j]
        for u in range(pl.cdiv(lead, nck)):
            att.m[u] = m_ref[u]
        acc = {}

        def project_heads(b, h0):
            rows = span(part * nb + b, R)
            a = acc[b] if h0 else jnp.where(g > 0, acc_ref[rows, :], 0.0)
            acc[b] = project(_merge_heads([(att.o[u], att.l[u]) for u in range(b * ng + h0, b * ng + h0 + eg)]), g, h0, a)
            if h0 + eg == ng:
                finish(rows, acc[b])

        prog = [((cfg["epos"], 4), finish_previous, (jnp.maximum(i - 1, 0),))]
        for j in range(units * nck):
            prog.append(((j, cfg["bpos"]), att.scores, (j + lead,)))
            prog.append(((j, 3), att.values, (j,)))
        for u in range(eg, units, eg):
            prog.append(((u * nck + cfg["epos"], 4), project_heads, divmod(u - eg, ng)))
        for _, fn, args in sorted(prog, key=lambda e: e[0]):
            fn(*args)
        hand_over(att, units * nck)
        for h in range(eg):
            tail_ref[0, h] = att.o[units - eg + h]
            tail_ref[1, h] = att.l[units - eg + h]
        part_ref[...] = acc[nb - 1]

        @pl.when(i > steps - parts2)
        def _():
            out_copy(part - 1).start()

        return carry

    if cfg['skip']:
        wait(group_copies(1))
        start([out_copy(p) for p in range(parts2 - 1)])
    else:
        lax.fori_loop(0, steps, attend_step, 0)
    out_copy(parts2 - 1).start()
    finish_previous(steps - 1)
    out_copy(parts2).start()
    wait([out_copy(p) for p in range(parts2 + 1)])


def make(R=64, CK=512, lead=7, epos=3, bpos=3.5, eg=4, ng=16, nb=4, R0=64, P0=512, R1=128, P1=1024, FC=384, skip=False, early=5, pa=13, pc=1, pn=8, flags=None):
    @jax.jit
    def fn(A_x, A_k_cache, A_v_cache, A_wq, A_wo, B_x, B_w_r, B_w_gate, B_w_up, B_w_down):
        B, S, D = A_x.shape
        Sk = A_k_cache.shape[2]
        cfg = dict(R=R, CK=CK, lead=lead, epos=epos, bpos=bpos, eg=eg, ng=ng, nb=nb, R0=R0, P0=P0, R1=R1, P1=P1,
                   FC=FC, Sk=Sk, skip=skip, early=early, pa=pa, pc=pc, pn=pn)
        panels = H * DH // QW
        Fp = (panels - 1) * (S // P1) * FC
        hbm = pl.BlockSpec(memory_space=pltpu.HBM)
        vmem, dma = pltpu.VMEM, pltpu.SemaphoreType.DMA
        return pl.pallas_call(
            functools.partial(_kernel, cfg=cfg),
            in_specs=[hbm] * 9,
            out_specs=hbm,
            out_shape=jax.ShapeDtypeStruct((B, S, D), A_x.dtype),
            scratch_shapes=[
                vmem((S, D), BF16), vmem((S, D), BF16), vmem((S, D), F32), vmem((S, D), F32), vmem((S, D), A_x.dtype),
                vmem((panels, S, QW), BF16), vmem((H, Sk, DH), BF16), vmem((H, Sk, DH), BF16),
                vmem((panels, D, QW), BF16), vmem((H * DH, D), BF16),
                vmem((Fp, D), BF16), vmem((Fp, D), BF16), vmem((Fp, D), BF16),
                vmem((lead, R, CK), F32), vmem((pl.cdiv(lead * CK, Sk), R, 128), F32), vmem((2, eg, R, DH), F32), vmem((R, D), F32),
                vmem((CAP, D), F32), vmem((R0, D), BF16), vmem((S // P0, 8, 128), F32), vmem((CAP, 128), I32),
                vmem((D,), BF16),
                dma((S // P0 + 1,)), dma((2,)), dma((panels,)), dma((4,)), dma((H // ng, 3)), dma((S // (nb * R) + 1,)),
            ],
            compiler_params=pltpu.CompilerParams(
                vmem_limit_bytes=112 * 1024 * 1024, internal_scratch_in_bytes=64 * 1024, flags=flags),
        )(A_x, A_k_cache, A_v_cache, A_wq, A_wo, B_w_r, B_w_gate.T, B_w_up.T, B_w_down)
    return fn


pallas_recurrent_scan__mha_block_cached__moe_arch_mod__prompt_kernel = make()
```

```python
import functools
import math

import jax
import jax.numpy as jnp
from jax import lax
import jax.experimental.pallas as pl
import jax.experimental.pallas.tpu as pltpu

F32 = jnp.float32
BF16 = jnp.bfloat16
I32 = jnp.int32

H, DH = 32, 128
CAP = 8
EPS = 1e-5
NT = (((1,), (1,)), ((), ()))
QW = 4 * DH


def _divmod(i, n):
    assert n & (n - 1) == 0
    return i >> (n.bit_length() - 1), i & (n - 1)


def _bf(x):
    return x.astype(BF16).astype(F32)


def _silu(x):
    h = 0.5 * x
    return h + h * jnp.tanh(h)


def _after(x, other):
    return jnp.where(other > jnp.inf, other, x)


def _layernorm(x, pace=None):
    d = x.shape[-1]
    x = x.astype(F32)
    if pace is not None:
        x = jnp.concatenate([_after(x[:, :128], pace), x[:, 128:]], axis=1)
    mu = jnp.sum(x, axis=-1, keepdims=True) * (1.0 / d)
    xc = x - mu
    var = jnp.sum(xc * xc, axis=-1, keepdims=True) * (1.0 / d)
    den = _bf(jnp.sqrt(_bf(_bf(var) + _bf(jnp.full_like(var, EPS)))))
    inv = pl.reciprocal(den, approx=True)
    inv = jnp.where(den == jnp.inf, 0.0, inv * (2.0 - den * inv))
    return (_bf(x - _bf(mu)) * inv).astype(BF16)


def _row_max(m):
    return jnp.broadcast_to(jnp.max(m, axis=-1, keepdims=True), m.shape)


class _Attention:
    def __init__(self, cfg, query, keys, vals):
        self.R, self.CK, self.nck = cfg["R"], cfg["CK"], cfg["Sk"] // cfg["CK"]
        self.query, self.keys, self.vals = query, keys, vals
        self.q, self.s, self.m, self.l, self.o = {}, {}, {}, {}, {}
        self.whole = set()

    def scores(self, j):
        u, c = divmod(j, self.nck)
        if u not in self.q:
            self.q[u] = self.query(u)
        s = self.s[j] = lax.dot_general(self.q[u], self.keys(u, c), NT, preferred_element_type=F32)
        m = jnp.maximum(s[:, :128], self.m[u]) if c else s[:, :128]
        for t in range(1, self.CK // 128):
            m = jnp.maximum(m, s[:, t * 128:(t + 1) * 128])
        self.m[u] = m

    def values(self, j):
        u, c = divmod(j, self.nck)
        if c == 0 and u not in self.whole:
            self.m[u] = _row_max(self.m[u])
        p = jnp.exp2(self.s[j] - jnp.concatenate([self.m[u]] * (self.CK // 128), axis=1))
        l = p[:, :128] + self.l[u] if c else p[:, :128]
        for t in range(1, self.CK // 128):
            l = l + p[:, t * 128:(t + 1) * 128]
        self.l[u] = l
        p = jnp.concatenate([p[:, :-128], jnp.minimum(p[:, -128:], l)], axis=1)
        o = jnp.dot(p.astype(BF16), self.vals(u, c), preferred_element_type=F32)
        self.o[u] = o + self.o[u] if c else o


def _merge_heads(pairs):
    heads = []
    for o, l in pairs:
        l = jnp.sum(l, axis=-1, keepdims=True)
        r = pl.reciprocal(l, approx=True)
        heads.append(o * (r * (2.0 - l * r)))
    return jnp.concatenate(heads, axis=1).astype(BF16)


def _kernel(x_hbm, k_hbm, v_hbm, wq_hbm, wo_hbm, wr_hbm, wg_hbm, wu_hbm, wd_hbm, out_hbm,
            x_ref, xn_ref, upd_ref, acc_ref, out_ref, q_ref, k_ref, v_ref, wq_ref, wo_ref,
            wg_ref, wu_ref, wd_ref, s_ref, m_ref, tail_ref, part_ref, head_ref, score_ref, xs_ref, y_ref, top_ref, wr_ref, wrf_ref,
            x_sem, q_sem, w_sem, p_sem, o_sem, *, cfg):
    S, D = x_ref.shape
    F = wg_hbm.shape[0]
    R, CK, ng, nb = cfg["R"], cfg["CK"], cfg["ng"], cfg["nb"]
    R0, P0, R1, P1, FC = cfg["R0"], cfg["P0"], cfg["R1"], cfg["P1"], cfg["FC"]
    panels, groups = H * DH // QW, H // ng
    parts0, parts1, parts2 = S // P0, S // P1, S // (nb * R)
    qscale = (DH ** -0.5) * math.log2(math.e)

    def span(i, n):
        return pl.ds(i * n if isinstance(i, int) else pl.multiple_of(i * n, n), n)

    def wq_copy(i):
        return pltpu.make_async_copy(wq_hbm.at[:, span(i, QW)], wq_ref.at[i], q_sem.at[i])

    def group_copies(g):
        return [pltpu.make_async_copy(k_hbm.at[0, span(g, ng)], k_ref.at[span(g, ng)], p_sem.at[g, 0]),
                pltpu.make_async_copy(v_hbm.at[0, span(g, ng)], v_ref.at[span(g, ng)], p_sem.at[g, 1]),
                pltpu.make_async_copy(wo_hbm.at[span(g, ng * DH)], wo_ref.at[span(g, ng * DH)], p_sem.at[g, 2])]

    def out_copy(i):
        rows = span(i, nb * R)
        if isinstance(i, int) and i >= parts2 - 1:
            rows = pl.ds(S - nb * R, (nb - 1) * R) if i < parts2 else pl.ds(S - R, R)
        return pltpu.make_async_copy(out_ref.at[rows], out_hbm.at[0, rows], o_sem.at[i])

    wr_copy = pltpu.make_async_copy(wr_hbm, wr_ref, w_sem.at[0])
    ffn_copies = [pltpu.make_async_copy(src, dst.at[:F], w_sem.at[i + 1])
                  for i, (src, dst) in enumerate([(wg_hbm, wg_ref), (wu_hbm, wu_ref), (wd_hbm, wd_ref)])]

    def start(copies):
        for c in copies:
            c.start()

    def wait(copies):
        for c in copies:
            c.wait()

    def project_q(xn, panel, rows):
        q = jnp.dot(xn, wq_ref[panel], preferred_element_type=F32)
        q_ref[panel, rows, :] = (q * qscale).astype(BF16)
        return q

    lane = lax.broadcasted_iota(I32, (8, 128), 1)
    per_part = P0 // 8
    nb0, early = P0 // R0, cfg["early"]

    def keep(i, normed):
        wr = wrf_ref[...].reshape(1, D)
        score = jnp.zeros((8, 128), F32)
        for b, xn in enumerate(normed):
            xn_ref[span(i * nb0 + b, R0), :] = xn
            upd_ref[span(i * nb0 + b, R0), :] = jnp.zeros((R0, D), F32)
            r = jnp.sum(xn.astype(F32) * wr, axis=-1, keepdims=True)
            for j in range(R0 // 8):
                score = jnp.where(lane % per_part == b * (R0 // 8) + j, r[j * 8:(j + 1) * 8], score)
        score_ref[i] = score

    edges = [0, early * R0] + [i * P0 + R0 for i in range(1, parts0)] + [S]
    x_copies = [pltpu.make_async_copy(x_hbm.at[0, a:b], x_ref.at[a:b], x_sem.at[i])
                for i, (a, b) in enumerate(zip(edges, edges[1:]))]

    def first_step():
        start([x_copies[0], wq_copy(0), x_copies[1], wq_copy(1)])
        for ref in (wg_ref, wu_ref, wd_ref):
            ref[F:, :] = jnp.zeros((ref.shape[0] - F, D), BF16)
        xs_ref[...] = jnp.zeros_like(xs_ref)
        y_ref[...] = jnp.zeros_like(y_ref)
        wait([x_copies[0]])
        normed = [_layernorm(x_ref[span(b, R0), :]) for b in range(early)]
        wait([wq_copy(0)])
        done = []
        for b in range(nb0):
            if b == early - 2:
                wait([x_copies[1]])
                start([wr_copy, x_copies[2]])
            if b >= early:
                normed.append(_layernorm(x_ref[span(b, R0), :]))
            done.append(project_q(normed[b], 0, span(b, R0)))
        wait([wq_copy(1), wr_copy])
        wrf_ref[...] = wr_ref[...].astype(F32)
        start(x_copies[3:])
        for b in range(nb0):
            project_q(normed[b], 1, span(b, R0))
        keep(0, normed)
        head_ref[...] = _layernorm(x_ref[span(nb0, R0), :])

    def norm_step(i):
        for j in range(1, parts0):
            pl.when(i == j)(x_copies[j + 1].wait)
        pl.when(i == 1)(functools.partial(start, [wq_copy(2), wq_copy(3)] + ffn_copies))
        pl.when(i == parts0 - 1)(functools.partial(start, [wq_copy(j) for j in range(4, panels)]))
        normed, done = [head_ref[...]], []

        def pace(b):
            n, per = cfg["pn"], QW // 128
            first = 2 * per * b - cfg["pa"]
            if first < 0:
                return None
            tiles = [divmod(first + j * cfg["pc"], per) for j in range(R0 // n)]
            return jnp.concatenate([done[d][j * n:(j + 1) * n, t * 128:(t + 1) * 128] for j, (d, t) in enumerate(tiles)], axis=0)

        for b in range(nb0):
            rows = span(i * nb0 + b, R0)
            if b:
                normed.append(_layernorm(x_ref[rows, :], pace(b)))
            done.append(project_q(normed[b], 0, rows))
            done.append(project_q(normed[b], 1, rows))
        keep(i, normed)
        head_ref[...] = _layernorm(x_ref[span(jnp.minimum(i + 1, parts0 - 1) * nb0, R0), :], pace(nb0))

    def route():
        tiles = []
        for t in range(S // 1024):
            ps = range(t * (128 // per_part), (t + 1) * (128 // per_part))
            tile = score_ref[ps[0]]
            for j, p in enumerate(ps[1:]):
                tile = jnp.where(lane // per_part == j + 1, score_ref[p], tile)
            tiles.append(tile)
        r = _bf(jnp.concatenate(tiles, axis=1))
        r = jnp.where(r == 0.0, 0.0, r)
        bits = pltpu.bitcast(r, I32) >> 16
        rank = jnp.where(r != r, 0, jnp.where(bits < 0, ~bits, bits + 0x8000))
        token = lax.broadcasted_iota(I32, r.shape, 1) * 8 + lax.broadcasted_iota(I32, r.shape, 0)
        key = pltpu.bitcast(((rank << 11) | (S - 1 - token)) + 0x08000000, F32)
        slot = lax.broadcasted_iota(I32, (CAP, 128), 0)
        top = jnp.zeros((CAP, 128), F32)
        for c in range(CAP):
            best = jnp.max(jnp.max(key, axis=0, keepdims=True), axis=1, keepdims=True)
            top = jnp.where(slot == c, best, top)
            key = jnp.where(key == best, 0.0, key)
        return pltpu.bitcast(top, I32) - 0x08000000

    def picked_tokens(top):
        return [(S - 1) - (top[c, 0] & (S - 1)) for c in range(CAP)]

    def gather(top):
        row = lax.broadcasted_iota(I32, (16, D), 0)
        slot = lax.broadcasted_iota(I32, (CAP, D), 0)
        xs = jnp.zeros((CAP, D), F32)
        for c, t in enumerate(picked_tokens(top)):
            near = xn_ref[span(t >> 4, 16), :].astype(F32)
            xs = jnp.where(slot == c, jnp.sum(jnp.where(row == (t & 15), near, 0.0), axis=0, keepdims=True), xs)
        return xs

    def panel_step(i):
        pair, part = _divmod(i + parts1, parts1)


        @pl.when(i == 0)
        def _():
            start(group_copies(0))

        pl.when(i == 1)(functools.partial(wait, ffn_copies))
        for j in range(1, panels // 2):
            pl.when(i == (j - 1) * parts1)(functools.partial(wait, [wq_copy(2 * j), wq_copy(2 * j + 1)]))

        hidden = pl.ds(pl.multiple_of(jnp.where(i == 0, wg_ref.shape[0] // FC - 1, i - 1) * FC, FC), FC)
        low = (lambda t: t) if cfg['f32'] else (lambda t: t.astype(BF16))
        xs = low(xs_ref[...])
        st = {}

        def ffn(n):
            k = n % (D // 128)
            cols = slice(k * 128, (k + 1) * 128)
            if n < 2 * (D // 128):
                ref = wg_ref if n < D // 128 else wu_ref
                t = lax.dot_general(xs[:, cols], ref[hidden, cols], NT, preferred_element_type=F32)
                st[n // (D // 128)] = t + st[n // (D // 128)] if k else t
            elif n < 3 * (D // 128):
                if k == 0:
                    st["h"] = low(_bf(_bf(_silu(_bf(st[0]))) * _bf(st[1])))
                st["y", k] = lax.dot_general(st["h"], wd_ref[hidden, cols], (((1,), (0,)), ((), ())), preferred_element_type=F32)

        for b in range(P1 // R1):
            rows = span(part * (P1 // R1) + b, R1)
            xn = xn_ref[rows, :]
            for half in range(2):
                project_q(xn, 2 * pair + half, rows)
                n = 2 * b + half
                if n != 2 * (D // 128):
                    ffn(n - (n > 2 * (D // 128)))
        top = route()
        top_ref[...] = top
        xs_ref[...] = gather(top)
        y_ref[...] += jnp.concatenate([st["y", k] for k in range(D // 128)], axis=1)

    nck, lead, eg = cfg["Sk"] // CK, cfg["lead"], cfg["eg"]
    ahead = lead + cfg["extra"]
    units, steps, per = nb * ng, groups * parts2, QW // DH

    def attention(i):
        after = min(i + 1, steps - 1) if isinstance(i, int) else jnp.minimum(i + 1, steps - 1)

        def place(u):
            step = i if u < units else after
            b, h = divmod(u % units, ng)
            g, part = _divmod(step, parts2)
            return g, span(part * nb + b, R), h

        def query(u):
            g, rows, h = place(u)
            return q_ref[g * (ng // per) + h // per, rows, (h % per) * DH:(h % per + 1) * DH]

        def cache(ref, u, c):
            g, _, h = place(u)
            return ref[g * ng + h, c * CK:(c + 1) * CK, :]

        return _Attention(cfg, query, functools.partial(cache, k_ref), functools.partial(cache, v_ref))

    def hand_over(att, first):
        for j in range(ahead):
            s_ref[j] = att.s[first + j]
        m_ref[0] = _row_max(att.m[first // nck])
        for u in range(1, pl.cdiv(ahead, nck)):
            m_ref[u] = att.m[first // nck + u]

    def project(o, g, h0, a):
        w = wo_ref[pl.ds(pl.multiple_of(g * (ng * DH), ng * DH) + h0 * DH, o.shape[1]), :]
        return jnp.dot(o, w, preferred_element_type=F32) + a

    def finish(rows, a):
        acc_ref[rows, :] = a
        gate = _silu(xn_ref[rows, :].astype(F32) + upd_ref[rows, :])
        out_ref[rows, :] = (x_ref[rows, :].astype(F32) + a * gate).astype(out_ref.dtype)

    def finish_previous(step):
        g, part = _divmod(step, parts2)
        finish(span(part * nb + nb - 1, R), project(_merge_heads([(tail_ref[0, h], tail_ref[1, h]) for h in range(eg)]),
                                                g, ng - eg, part_ref[...]))

    def prime():
        wait(group_copies(0))
        start([c for g in range(1, groups) for c in group_copies(g)])
        att = attention(0)
        for j in range(ahead):
            att.scores(j)
        hand_over(att, 0)
        tail_ref[...] = jnp.ones_like(tail_ref)
        part_ref[...] = jnp.zeros_like(part_ref)
        top = top_ref[...]
        rank = top >> 11
        r_sel = pltpu.bitcast(jnp.where(rank < 0x8000, ~rank, rank - 0x8000) << 16, F32)
        y = _bf(_bf(y_ref[...]) * _bf(jax.nn.sigmoid(r_sel[:, :1])))
        for c, t in enumerate(picked_tokens(top)):
            upd_ref[pl.ds(t, 1), :] = y[c:c + 1, :]

    def attend_step(i):
        g, part = _divmod(i, parts2)
        for nxt in range(1, groups):
            pl.when(i == nxt * parts2 - 1)(functools.partial(wait, group_copies(nxt)))

        att = attention(i)
        for j in range(ahead):
            att.s[j] = s_ref[j]
        for u in range(pl.cdiv(ahead, nck)):
            att.m[u] = m_ref[u]
        att.whole.add(0)
        acc = {}

        def project_heads(b, h0):
            rows = span(part * nb + b, R)
            a = acc[b] if h0 else jnp.where(g > 0, acc_ref[rows, :], 0.0)
            acc[b] = project(_merge_heads([(att.o[u], att.l[u]) for u in range(b * ng + h0, b * ng + h0 + eg)]), g, h0, a)
            if h0 + eg == ng:
                finish(rows, acc[b])

        prog = [((cfg["epos"], 4), finish_previous, (jnp.maximum(i - 1, 0),))]
        for j in range(units * nck):
            prog.append(((j + ahead - lead, cfg["bpos"]), att.scores, (j + ahead,)))
            prog.append(((j, 3), att.values, (j,)))
        for u in range(eg, units, eg):
            prog.append(((u * nck + cfg["epos"], 4), project_heads, divmod(u - eg, ng)))
        for _, fn, args in sorted(prog, key=lambda e: e[0]):
            fn(*args)
        hand_over(att, units * nck)
        for h in range(eg):
            tail_ref[0, h] = att.o[units - eg + h]
            tail_ref[1, h] = att.l[units - eg + h]
        part_ref[...] = acc[nb - 1]

        @pl.when(i > steps - parts2)
        def _():
            out_copy(part - 1).start()

    t1 = parts0 + (panels // 2 - 1) * parts1

    @pl.loop(0, t1 + steps)
    def _(t):
        @pl.when(t < t1)
        def _():
            pl.when(t == 0)(first_step)
            pl.when((t > 0) & (t < parts0))(lambda: norm_step(t))
            pl.when(t >= parts0)(lambda: panel_step(t - parts0))
            pl.when(t == t1 - 1)(prime)

        pl.when(t >= t1)(lambda: attend_step(t - t1))

    out_copy(parts2 - 1).start()
    finish_previous(steps - 1)
    out_copy(parts2).start()
    wait([out_copy(p) for p in range(parts2 + 1)])


def make(R=64, CK=512, lead=7, epos=3, bpos=3.5, extra=1, f32=True, eg=4, ng=16, nb=4, R0=64, P0=512, R1=128, P1=1024, FC=384, skip=False, early=5, pa=13, pc=1, pn=8, flags=None):
    @jax.jit
    def fn(A_x, A_k_cache, A_v_cache, A_wq, A_wo, B_x, B_w_r, B_w_gate, B_w_up, B_w_down):
        B, S, D = A_x.shape
        Sk = A_k_cache.shape[2]
        cfg = dict(R=R, CK=CK, lead=lead, epos=epos, bpos=bpos, extra=extra, f32=f32, eg=eg, ng=ng, nb=nb, R0=R0, P0=P0, R1=R1, P1=P1,
                   FC=FC, Sk=Sk, skip=skip, early=early, pa=pa, pc=pc, pn=pn)
        panels = H * DH // QW
        Fp = (panels // 2 - 1) * (S // P1) * FC
        hbm = pl.BlockSpec(memory_space=pltpu.HBM)
        vmem, dma = pltpu.VMEM, pltpu.SemaphoreType.DMA
        return pl.pallas_call(
            functools.partial(_kernel, cfg=cfg),
            in_specs=[hbm] * 9,
            out_specs=hbm,
            out_shape=jax.ShapeDtypeStruct((B, S, D), A_x.dtype),
            scratch_shapes=[
                vmem((S, D), BF16), vmem((S, D), BF16), vmem((S, D), F32), vmem((S, D), F32), vmem((S, D), A_x.dtype),
                vmem((panels, S, QW), BF16), vmem((H, Sk, DH), BF16), vmem((H, Sk, DH), BF16),
                vmem((panels, D, QW), BF16), vmem((H * DH, D), BF16),
                vmem((Fp, D), BF16), vmem((Fp, D), BF16), vmem((Fp, D), BF16),
                vmem((lead + extra, R, CK), F32), vmem((pl.cdiv((lead + extra) * CK, Sk), R, 128), F32), vmem((2, eg, R, DH), F32), vmem((R, D), F32),
                vmem((R0, D), BF16), vmem((S // P0, 8, 128), F32), vmem((CAP, D), F32), vmem((CAP, D), F32), vmem((CAP, 128), I32),
                vmem((D,), BF16), vmem((D,), F32),
                dma((S // P0 + 1,)), dma((panels,)), dma((4,)), dma((H // ng, 3)), dma((S // (nb * R) + 1,)),
            ],
            compiler_params=pltpu.CompilerParams(
                vmem_limit_bytes=112 * 1024 * 1024, internal_scratch_in_bytes=64 * 1024, flags=flags),
        )(A_x, A_k_cache, A_v_cache, A_wq, A_wo, B_w_r, B_w_gate.T, B_w_up.T, B_w_down)
    return fn


pallas_recurrent_scan__mha_block_cached__moe_arch_mod__prompt_kernel = make()
```

```python
import functools
import math

import jax
import jax.numpy as jnp
from jax import lax
import jax.experimental.pallas as pl
import jax.experimental.pallas.tpu as pltpu

F32 = jnp.float32
BF16 = jnp.bfloat16
I32 = jnp.int32
NN = (((1,), (0,)), ((), ()))
NT = (((1,), (1,)), ((), ()))

H, DH = 32, 128
CAP = 8
EPS = 1e-5

QW = 4 * DH
R = 64
NORM_ROWS = 512
EARLY = 5
PROJ_ROWS = 1024
PROJ_BLOCK = 128
FFN_CHUNK = 384
CK = 512
HEADS = 16
BLOCKS = 4
MERGE = 4
LEAD = 7
AHEAD = 8
LAG = 3


def _divmod(i, n):
    assert n & (n - 1) == 0
    return i >> (n.bit_length() - 1), i & (n - 1)


def _span(i, n):
    return pl.ds(i * n if isinstance(i, int) else pl.multiple_of(i * n, n), n)


def _start(copies):
    for c in copies:
        c.start()


def _wait(copies):
    for c in copies:
        c.wait()


def _bf(x):
    return x.astype(BF16).astype(F32)


def _silu(x):
    h = 0.5 * x
    return h + h * jnp.tanh(h)


def _reciprocal(d):
    r = pl.reciprocal(d, approx=True)
    return r * (2.0 - d * r)


def _after(x, other):
    return jnp.where(other > jnp.inf, other, x)


def _layernorm(x, pace=None):
    d = x.shape[-1]
    x = x.astype(F32)
    if pace is not None:
        x = jnp.concatenate([_after(x[:, :128], pace), x[:, 128:]], axis=1)
    mu = jnp.sum(x, axis=-1, keepdims=True) * (1.0 / d)
    xc = x - mu
    var = jnp.sum(xc * xc, axis=-1, keepdims=True) * (1.0 / d)
    den = _bf(jnp.sqrt(_bf(_bf(var) + _bf(jnp.full_like(var, EPS)))))
    inv = jnp.where(den == jnp.inf, 0.0, _reciprocal(den))
    return (_bf(x - _bf(mu)) * inv).astype(BF16)


def _row_max(m):
    return jnp.broadcast_to(jnp.max(m, axis=-1, keepdims=True), m.shape)


class _Attention:
    def __init__(self, chunks, query, keys, vals):
        self.chunks, self.query, self.keys, self.vals = chunks, query, keys, vals
        self.q, self.s, self.m, self.l, self.o = {}, {}, {}, {}, {}
        self.whole = set()

    def scores(self, j):
        u, c = divmod(j, self.chunks)
        if u not in self.q:
            self.q[u] = self.query(u)
        s = self.s[j] = lax.dot_general(self.q[u], self.keys(u, c), NT, preferred_element_type=F32)
        m = jnp.maximum(s[:, :128], self.m[u]) if c else s[:, :128]
        for t in range(1, CK // 128):
            m = jnp.maximum(m, s[:, t * 128:(t + 1) * 128])
        self.m[u] = m

    def values(self, j):
        u, c = divmod(j, self.chunks)
        if c == 0 and u not in self.whole:
            self.m[u] = _row_max(self.m[u])
        p = jnp.exp2(self.s[j] - jnp.concatenate([self.m[u]] * (CK // 128), axis=1))
        l = p[:, :128] + self.l[u] if c else p[:, :128]
        for t in range(1, CK // 128):
            l = l + p[:, t * 128:(t + 1) * 128]
        self.l[u] = l
        p = jnp.concatenate([p[:, :-128], jnp.minimum(p[:, -128:], l)], axis=1)
        o = jnp.dot(p.astype(BF16), self.vals(u, c), preferred_element_type=F32)
        self.o[u] = o + self.o[u] if c else o


def _merge_heads(pairs):
    heads = [o * _reciprocal(jnp.sum(l, axis=-1, keepdims=True)) for o, l in pairs]
    return jnp.concatenate(heads, axis=1).astype(BF16)


def _kernel(x_hbm, k_hbm, v_hbm, wq_hbm, wo_hbm, wr_hbm, wg_hbm, wu_hbm, wd_hbm, out_hbm,
            x_ref, xn_ref, upd_ref, acc_ref, out_ref, q_ref, k_ref, v_ref, wq_ref, wo_ref,
            wg_ref, wu_ref, wd_ref, s_ref, m_ref, tail_ref, part_ref, head_ref, score_ref,
            xs_ref, y_ref, top_ref, wr_ref, wrf_ref,
            x_sem, h_sem, q_sem, w_sem, p_sem, o_sem):
    S, D = x_ref.shape
    F = wg_hbm.shape[0]
    panels, groups, chunks = H * DH // QW, H // HEADS, k_ref.shape[1] // CK
    norm_parts, proj_parts, parts = S // NORM_ROWS, S // PROJ_ROWS, S // (BLOCKS * R)
    qscale = (DH ** -0.5) * math.log2(math.e)

    edges = [0, EARLY * R] + [i * NORM_ROWS + R for i in range(1, norm_parts)] + [S]
    x_copies = [pltpu.make_async_copy(x_hbm.at[0, a:b], x_ref.at[a:b], x_sem.at[i])
                for i, (a, b) in enumerate(zip(edges, edges[1:]))]
    wr_copy = pltpu.make_async_copy(wr_hbm, wr_ref, w_sem.at[0])
    ffn_copies = [pltpu.make_async_copy(src, dst.at[:F], w_sem.at[i + 1])
                  for i, (src, dst) in enumerate([(wg_hbm, wg_ref), (wu_hbm, wu_ref), (wd_hbm, wd_ref)])]

    def wq_copy(i):
        return pltpu.make_async_copy(wq_hbm.at[:, _span(i, QW)], wq_ref.at[i], q_sem.at[i])

    def group_copies(g):
        heads, rows = _span(g, HEADS), _span(g, HEADS * DH)
        return [pltpu.make_async_copy(k_hbm.at[0, heads], k_ref.at[heads], p_sem.at[g, 0]),
                pltpu.make_async_copy(v_hbm.at[0, heads], v_ref.at[heads], p_sem.at[g, 1]),
                pltpu.make_async_copy(wo_hbm.at[rows], wo_ref.at[rows], p_sem.at[g, 2])]

    def out_copy(i):
        rows = _span(i, BLOCKS * R)
        if isinstance(i, int) and i >= parts - 1:
            rows = pl.ds(S - BLOCKS * R, (BLOCKS - 1) * R) if i < parts else pl.ds(S - R, R)
        return pltpu.make_async_copy(out_ref.at[rows], out_hbm.at[0, rows], o_sem.at[i])

    lane = lax.broadcasted_iota(I32, (8, 128), 1)
    per_part = NORM_ROWS // 8
    nblk = NORM_ROWS // R

    def project_q(xn, panel, rows, cols=slice(None)):
        q = jnp.dot(xn, wq_ref[panel, :, cols], preferred_element_type=F32)
        q_ref[panel, rows, cols] = (q * qscale).astype(BF16)
        return q

    def keep(i, normed):
        wr = wrf_ref[...].reshape(1, D)
        score = jnp.zeros((8, 128), F32)
        for b, xn in enumerate(normed):
            xn_ref[_span(i * nblk + b, R), :] = xn
            upd_ref[_span(i * nblk + b, R), :] = jnp.zeros((R, D), F32)
            r = jnp.sum(xn.astype(F32) * wr, axis=-1, keepdims=True)
            for j in range(R // 8):
                score = jnp.where(lane % per_part == b * (R // 8) + j, r[j * 8:(j + 1) * 8], score)
        score_ref[i] = score

    def first_step():
        halves = [slice(0, QW // 2), slice(QW // 2, QW)]
        pieces = [pltpu.make_async_copy(wq_hbm.at[:, c], wq_ref.at[0, :, c], h_sem.at[i])
                  for i, c in enumerate(halves)]
        _start([x_copies[0]] + pieces + [x_copies[1]])
        for ref in (wg_ref, wu_ref, wd_ref):
            ref[F:, :] = jnp.zeros((ref.shape[0] - F, D), BF16)
        xs_ref[...] = jnp.zeros_like(xs_ref)
        y_ref[...] = jnp.zeros_like(y_ref)
        x_copies[0].wait()
        normed = [_layernorm(x_ref[_span(b, R), :]) for b in range(EARLY)]
        pieces[0].wait()
        wq_copy(1).start()
        for b in range(EARLY):
            project_q(normed[b], 0, _span(b, R), halves[0])
        pieces[1].wait()
        for b in range(EARLY):
            if b == EARLY // 2:
                x_copies[1].wait()
                wr_copy.start()
            project_q(normed[b], 0, _span(b, R), halves[1])
        for b in range(EARLY, nblk):
            normed.append(_layernorm(x_ref[_span(b, R), :]))
            project_q(normed[b], 0, _span(b, R))
        _wait([wq_copy(1), wr_copy])
        wrf_ref[...] = wr_ref[...].astype(F32)
        _start(x_copies[2:])
        for b in range(nblk):
            project_q(normed[b], 1, _span(b, R))
        keep(0, normed)
        head_ref[...] = _layernorm(x_ref[_span(nblk, R), :])

    def norm_step(i):
        for j in range(1, norm_parts):
            pl.when(i == j)(x_copies[j + 1].wait)
        pl.when(i == 1)(functools.partial(_start, [wq_copy(2), wq_copy(3)] + ffn_copies))
        pl.when(i == norm_parts - 1)(functools.partial(_start, [wq_copy(j) for j in range(4, panels)]))
        normed, done = [head_ref[...]], []

        def pace(b):
            if b < 2:
                return None
            tiles = [divmod(3 + j, QW // 128) for j in range(R // 16)]
            return jnp.concatenate([done[2 * (b - 2) + d][j * 16:(j + 1) * 16, t * 128:(t + 1) * 128]
                                    for j, (d, t) in enumerate(tiles)], axis=0)

        for b in range(nblk):
            rows = _span(i * nblk + b, R)
            if b:
                normed.append(_layernorm(x_ref[rows, :], pace(b)))
            done.append(project_q(normed[b], 0, rows))
            done.append(project_q(normed[b], 1, rows))
        keep(i, normed)
        following = jnp.minimum(i + 1, norm_parts - 1) * nblk
        head_ref[...] = _layernorm(x_ref[_span(following, R), :], pace(nblk))

    def route():
        tiles, side = [], 128 // per_part
        for t in range(norm_parts // side):
            tile = score_ref[t * side]
            for j in range(1, side):
                tile = jnp.where(lane // per_part == j, score_ref[t * side + j], tile)
            tiles.append(tile)
        r = _bf(jnp.concatenate(tiles, axis=1))
        r = jnp.where(r == 0.0, 0.0, r)
        bits = pltpu.bitcast(r, I32) >> 16
        rank = jnp.where(r != r, 0, jnp.where(bits < 0, ~bits, bits + 0x8000))
        token = lax.broadcasted_iota(I32, r.shape, 1) * 8 + lax.broadcasted_iota(I32, r.shape, 0)
        key = pltpu.bitcast(((rank << 11) | (S - 1 - token)) + 0x08000000, F32)
        slot = lax.broadcasted_iota(I32, (CAP, 128), 0)
        top = jnp.zeros((CAP, 128), F32)
        for c in range(CAP):
            best = jnp.max(jnp.max(key, axis=0, keepdims=True), axis=1, keepdims=True)
            top = jnp.where(slot == c, best, top)
            key = jnp.where(key == best, 0.0, key)
        return pltpu.bitcast(top, I32) - 0x08000000

    def tokens(top):
        return [(S - 1) - (top[c, 0] & (S - 1)) for c in range(CAP)]

    def gather(top):
        row = lax.broadcasted_iota(I32, (16, D), 0)
        slot = lax.broadcasted_iota(I32, (CAP, D), 0)
        xs = jnp.zeros((CAP, D), F32)
        for c, t in enumerate(tokens(top)):
            near = xn_ref[_span(t >> 4, 16), :].astype(F32)
            xs = jnp.where(slot == c, jnp.sum(jnp.where(row == (t & 15), near, 0.0), axis=0, keepdims=True), xs)
        return xs

    def panel_step(i):
        pair, part = _divmod(i + proj_parts, proj_parts)
        pl.when(i == 0)(functools.partial(_start, group_copies(0)))
        pl.when(i == 1)(functools.partial(_wait, ffn_copies))
        for j in range(1, panels // 2):
            pl.when(i == (j - 1) * proj_parts)(functools.partial(_wait, [wq_copy(2 * j), wq_copy(2 * j + 1)]))

        hidden = _span(jnp.where(i == 0, wg_ref.shape[0] // FFN_CHUNK - 1, i - 1), FFN_CHUNK)
        xs = xs_ref[...]
        tiles = D // 128
        st = {}

        def swiglu(stage, k):
            cols = slice(k * 128, (k + 1) * 128)
            if stage < 2:
                t = lax.dot_general(xs[:, cols], (wg_ref, wu_ref)[stage][hidden, cols], NT, preferred_element_type=F32)
                st[stage] = t + st[stage] if k else t
            else:
                if k == 0:
                    st["h"] = _bf(_bf(_silu(_bf(st[0]))) * _bf(st[1]))
                st["y", k] = lax.dot_general(st["h"], wd_ref[hidden, cols], NN, preferred_element_type=F32)

        small = [(stage, k) for stage in range(3) for k in range(tiles)]
        small.insert(2 * tiles, None)
        assert len(small) == 2 * PROJ_ROWS // PROJ_BLOCK
        for b in range(PROJ_ROWS // PROJ_BLOCK):
            rows = _span(part * (PROJ_ROWS // PROJ_BLOCK) + b, PROJ_BLOCK)
            xn = xn_ref[rows, :]
            for half in range(2):
                project_q(xn, 2 * pair + half, rows)
                if small[2 * b + half]:
                    swiglu(*small[2 * b + half])
        top = route()
        top_ref[...] = top
        xs_ref[...] = gather(top)
        y_ref[...] += jnp.concatenate([st["y", k] for k in range(tiles)], axis=1)

    units, steps, per_panel = BLOCKS * HEADS, groups * parts, QW // DH

    def attention(i):
        after = min(i + 1, steps - 1) if isinstance(i, int) else jnp.minimum(i + 1, steps - 1)

        def place(u):
            b, h = divmod(u % units, HEADS)
            g, part = _divmod(i if u < units else after, parts)
            return g, _span(part * BLOCKS + b, R), h

        def query(u):
            g, rows, h = place(u)
            panel, col = divmod(h, per_panel)
            return q_ref[g * (HEADS // per_panel) + panel, rows, col * DH:(col + 1) * DH]

        def cache(ref, u, c):
            g, _, h = place(u)
            return ref[g * HEADS + h, c * CK:(c + 1) * CK, :]

        return _Attention(chunks, query, functools.partial(cache, k_ref), functools.partial(cache, v_ref))

    def hand_over(att, first):
        for j in range(AHEAD):
            s_ref[j] = att.s[first + j]
        m_ref[0] = _row_max(att.m[first // chunks])
        for u in range(1, pl.cdiv(AHEAD, chunks)):
            m_ref[u] = att.m[first // chunks + u]

    def project_o(o, g, h0, a):
        w = wo_ref[pl.ds(pl.multiple_of(g * (HEADS * DH), HEADS * DH) + h0 * DH, MERGE * DH), :]
        return jnp.dot(o, w, preferred_element_type=F32) + a

    def finish(rows, a):
        acc_ref[rows, :] = a
        gate = _silu(xn_ref[rows, :].astype(F32) + upd_ref[rows, :])
        out_ref[rows, :] = (x_ref[rows, :].astype(F32) + a * gate).astype(out_ref.dtype)

    def finish_step(step):
        g, part = _divmod(step, parts)
        o = _merge_heads([(tail_ref[0, h], tail_ref[1, h]) for h in range(MERGE)])
        finish(_span(part * BLOCKS + BLOCKS - 1, R), project_o(o, g, HEADS - MERGE, part_ref[...]))

    def prime():
        _wait(group_copies(0))
        _start([c for g in range(1, groups) for c in group_copies(g)])
        att = attention(0)
        for j in range(AHEAD):
            att.scores(j)
        hand_over(att, 0)
        tail_ref[...] = jnp.ones_like(tail_ref)
        part_ref[...] = jnp.zeros_like(part_ref)
        top = top_ref[...]
        rank = top >> 11
        r_sel = pltpu.bitcast(jnp.where(rank < 0x8000, ~rank, rank - 0x8000) << 16, F32)
        y = _bf(_bf(y_ref[...]) * _bf(jax.nn.sigmoid(r_sel[:, :1])))
        for c, t in enumerate(tokens(top)):
            upd_ref[pl.ds(t, 1), :] = y[c:c + 1, :]

    def attend_step(i):
        g, part = _divmod(i, parts)
        for nxt in range(1, groups):
            pl.when(i == nxt * parts - 1)(functools.partial(_wait, group_copies(nxt)))
        att = attention(i)
        for j in range(AHEAD):
            att.s[j] = s_ref[j]
        for u in range(pl.cdiv(AHEAD, chunks)):
            att.m[u] = m_ref[u]
        att.whole.add(0)
        acc = {}

        def project_heads(b, h0):
            rows, u0 = _span(part * BLOCKS + b, R), b * HEADS + h0
            a = acc[b] if h0 else jnp.where(g > 0, acc_ref[rows, :], 0.0)
            acc[b] = project_o(_merge_heads([(att.o[u], att.l[u]) for u in range(u0, u0 + MERGE)]), g, h0, a)
            if h0 + MERGE == HEADS:
                finish(rows, acc[b])

        program = [((LAG, 2), finish_step, (jnp.maximum(i - 1, 0),))]
        for j in range(units * chunks):
            program.append(((j, 0), att.values, (j,)))
            program.append(((j + AHEAD - LEAD, 1), att.scores, (j + AHEAD,)))
        for u in range(MERGE, units, MERGE):
            program.append(((u * chunks + LAG, 2), project_heads, divmod(u - MERGE, HEADS)))
        for _, fn, args in sorted(program, key=lambda e: e[0]):
            fn(*args)
        hand_over(att, units * chunks)
        for h in range(MERGE):
            tail_ref[0, h] = att.o[units - MERGE + h]
            tail_ref[1, h] = att.l[units - MERGE + h]
        part_ref[...] = acc[BLOCKS - 1]

        @pl.when(i > steps - parts)
        def _():
            out_copy(part - 1).start()

    projected = norm_parts + (panels // 2 - 1) * proj_parts

    @pl.loop(0, projected + steps)
    def _(t):
        @pl.when(t < projected)
        def _():
            pl.when(t == 0)(first_step)
            pl.when((t > 0) & (t < norm_parts))(lambda: norm_step(t))
            pl.when(t >= norm_parts)(lambda: panel_step(t - norm_parts))
            pl.when(t == projected - 1)(prime)

        pl.when(t >= projected)(lambda: attend_step(t - projected))

    out_copy(parts - 1).start()
    finish_step(steps - 1)
    out_copy(parts).start()
    _wait([out_copy(p) for p in range(parts + 1)])


@jax.jit
def pallas_recurrent_scan__mha_block_cached__moe_arch_mod__prompt_kernel(
    A_x: jax.Array,
    A_k_cache: jax.Array,
    A_v_cache: jax.Array,
    A_wq: jax.Array,
    A_wo: jax.Array,
    B_x: jax.Array,
    B_w_r: jax.Array,
    B_w_gate: jax.Array,
    B_w_up: jax.Array,
    B_w_down: jax.Array,
):
    del B_x
    B, S, D = A_x.shape
    Sk = A_k_cache.shape[2]
    panels = H * DH // QW
    hidden = (panels // 2 - 1) * (S // PROJ_ROWS) * FFN_CHUNK
    assert B == 1 and S == 2048 and Sk % CK == 0 and B_w_gate.shape[1] <= hidden - FFN_CHUNK
    hbm = pl.BlockSpec(memory_space=pltpu.HBM)
    vmem, dma = pltpu.VMEM, pltpu.SemaphoreType.DMA
    scratch = [
        vmem((S, D), BF16), vmem((S, D), BF16), vmem((S, D), F32), vmem((S, D), F32), vmem((S, D), A_x.dtype),
        vmem((panels, S, QW), BF16), vmem((H, Sk, DH), BF16), vmem((H, Sk, DH), BF16),
        vmem((panels, D, QW), BF16), vmem((H * DH, D), BF16),
        vmem((hidden, D), BF16), vmem((hidden, D), BF16), vmem((hidden, D), BF16),
        vmem((AHEAD, R, CK), F32), vmem((pl.cdiv(AHEAD * CK, Sk), R, 128), F32),
        vmem((2, MERGE, R, DH), F32), vmem((R, D), F32), vmem((R, D), BF16), vmem((S // NORM_ROWS, 8, 128), F32),
        vmem((CAP, D), F32), vmem((CAP, D), F32), vmem((CAP, 128), I32), vmem((D,), BF16), vmem((D,), F32),
        dma((S // NORM_ROWS + 1,)), dma((2,)), dma((panels,)), dma((4,)), dma((H // HEADS, 3)),
        dma((S // (BLOCKS * R) + 1,)),
    ]
    return pl.pallas_call(
        _kernel,
        in_specs=[hbm] * 9,
        out_specs=hbm,
        out_shape=jax.ShapeDtypeStruct((B, S, D), A_x.dtype),
        scratch_shapes=scratch,
        compiler_params=pltpu.CompilerParams(
            vmem_limit_bytes=112 * 1024 * 1024, internal_scratch_in_bytes=64 * 1024),
    )(A_x, A_k_cache, A_v_cache, A_wq, A_wo, B_w_r, B_w_gate.T, B_w_up.T, B_w_down)
```

```python
import functools
import math

import jax
import jax.numpy as jnp
from jax import lax
import jax.experimental.pallas as pl
import jax.experimental.pallas.tpu as pltpu

F32 = jnp.float32
BF16 = jnp.bfloat16
I32 = jnp.int32
NN = (((1,), (0,)), ((), ()))
NT = (((1,), (1,)), ((), ()))

H, DH = 32, 128
CAP = 8
EPS = 1e-5

QW = 4 * DH
R = 64
NORM_ROWS = 512
EARLY = 5
PROJ_ROWS = 1024
PROJ_BLOCK = 128
FFN_CHUNK = 384
CK = 512
HEADS = 16
BLOCKS = 4
MERGE = 4
LEAD = 7
AHEAD = 8
LAG = 3


def _divmod(i, n):
    assert n & (n - 1) == 0
    return i >> (n.bit_length() - 1), i & (n - 1)


def _span(i, n):
    return pl.ds(i * n if isinstance(i, int) else pl.multiple_of(i * n, n), n)


def _start(copies):
    for c in copies:
        c.start()


def _wait(copies):
    for c in copies:
        c.wait()


def _loop_with_wait(n, body, at, copies):
    @pl.loop(0, 2)
    def _(half):
        pl.when(half == 1)(functools.partial(_wait, copies))
        pl.loop(half * at, jnp.where(half == 0, at, n))(body)


def _bf(x):
    return x.astype(BF16).astype(F32)


def _silu(x):
    h = 0.5 * x
    return h + h * jnp.tanh(h)


def _reciprocal(d):
    r = pl.reciprocal(d, approx=True)
    return r * (2.0 - d * r)


def _after(x, other):
    return jnp.where(other > jnp.inf, other, x)


def _layernorm(x, pace=None):
    d = x.shape[-1]
    x = x.astype(F32)
    if pace is not None:
        x = jnp.concatenate([_after(x[:, :128], pace), x[:, 128:]], axis=1)
    mu = jnp.sum(x, axis=-1, keepdims=True) * (1.0 / d)
    xc = x - mu
    var = jnp.sum(xc * xc, axis=-1, keepdims=True) * (1.0 / d)
    den = _bf(jnp.sqrt(_bf(_bf(var) + _bf(jnp.full_like(var, EPS)))))
    inv = jnp.where(den == jnp.inf, 0.0, _reciprocal(den))
    return (_bf(x - _bf(mu)) * inv).astype(BF16)


def _row_max(m):
    return jnp.broadcast_to(jnp.max(m, axis=-1, keepdims=True), m.shape)


class _Attention:
    def __init__(self, chunks, query, keys, vals):
        self.chunks, self.query, self.keys, self.vals = chunks, query, keys, vals
        self.q, self.s, self.m, self.l, self.o = {}, {}, {}, {}, {}
        self.whole = set()

    def scores(self, j):
        u, c = divmod(j, self.chunks)
        if u not in self.q:
            self.q[u] = self.query(u)
        s = self.s[j] = lax.dot_general(self.q[u], self.keys(u, c), NT, preferred_element_type=F32)
        m = jnp.maximum(s[:, :128], self.m[u]) if c else s[:, :128]
        for t in range(1, CK // 128):
            m = jnp.maximum(m, s[:, t * 128:(t + 1) * 128])
        self.m[u] = m

    def values(self, j):
        u, c = divmod(j, self.chunks)
        if c == 0 and u not in self.whole:
            self.m[u] = _row_max(self.m[u])
        p = jnp.exp2(self.s[j] - jnp.concatenate([self.m[u]] * (CK // 128), axis=1))
        l = p[:, :128] + self.l[u] if c else p[:, :128]
        for t in range(1, CK // 128):
            l = l + p[:, t * 128:(t + 1) * 128]
        self.l[u] = l
        p = jnp.concatenate([p[:, :-128], jnp.minimum(p[:, -128:], l)], axis=1)
        o = jnp.dot(p.astype(BF16), self.vals(u, c), preferred_element_type=F32)
        self.o[u] = o + self.o[u] if c else o


def _merge_heads(pairs):
    heads = [o * _reciprocal(jnp.sum(l, axis=-1, keepdims=True)) for o, l in pairs]
    return jnp.concatenate(heads, axis=1).astype(BF16)


def _kernel(x_hbm, k_hbm, v_hbm, wq_hbm, wo_hbm, wr_hbm, wg_hbm, wu_hbm, wd_hbm, out_hbm,
            x_ref, xn_ref, upd_ref, acc_ref, out_ref, q_ref, k_ref, v_ref, wq_ref, wo_ref,
            wg_ref, wu_ref, wd_ref, s_ref, m_ref, tail_ref, part_ref, head_ref, score_ref,
            xs_ref, y_ref, top_ref, wr_ref, wrf_ref,
            x_sem, h_sem, q_sem, w_sem, p_sem, o_sem):
    S, D = x_ref.shape
    F = wg_hbm.shape[0]
    panels, groups, chunks = H * DH // QW, H // HEADS, k_ref.shape[1] // CK
    norm_parts, proj_parts, parts = S // NORM_ROWS, S // PROJ_ROWS, S // (BLOCKS * R)
    qscale = (DH ** -0.5) * math.log2(math.e)

    edges = [0, EARLY * R] + [i * NORM_ROWS + R for i in range(1, norm_parts)] + [S]
    x_copies = [pltpu.make_async_copy(x_hbm.at[0, a:b], x_ref.at[a:b], x_sem.at[i])
                for i, (a, b) in enumerate(zip(edges, edges[1:]))]
    wr_copy = pltpu.make_async_copy(wr_hbm, wr_ref, w_sem.at[0])
    ffn_copies = [pltpu.make_async_copy(src, dst.at[:F], w_sem.at[i + 1])
                  for i, (src, dst) in enumerate([(wg_hbm, wg_ref), (wu_hbm, wu_ref), (wd_hbm, wd_ref)])]

    def wq_copy(i):
        return pltpu.make_async_copy(wq_hbm.at[:, _span(i, QW)], wq_ref.at[i], q_sem.at[i])

    def group_copies(g):
        heads, rows = _span(g, HEADS), _span(g, HEADS * DH)
        return [pltpu.make_async_copy(k_hbm.at[0, heads], k_ref.at[heads], p_sem.at[g, 0]),
                pltpu.make_async_copy(v_hbm.at[0, heads], v_ref.at[heads], p_sem.at[g, 1]),
                pltpu.make_async_copy(wo_hbm.at[rows], wo_ref.at[rows], p_sem.at[g, 2])]

    def out_copy(i):
        rows = _span(i, BLOCKS * R)
        if isinstance(i, int) and i >= parts - 1:
            rows = pl.ds(S - BLOCKS * R, (BLOCKS - 1) * R) if i < parts else pl.ds(S - R, R)
        return pltpu.make_async_copy(out_ref.at[rows], out_hbm.at[0, rows], o_sem.at[i])

    lane = lax.broadcasted_iota(I32, (8, 128), 1)
    per_part = NORM_ROWS // 8
    nblk = NORM_ROWS // R

    def project_q(xn, panel, rows, cols=slice(None)):
        q = jnp.dot(xn, wq_ref[panel, :, cols], preferred_element_type=F32)
        q_ref[panel, rows, cols] = (q * qscale).astype(BF16)
        return q

    def keep(i, normed):
        wr = wrf_ref[...].reshape(1, D)
        score = jnp.zeros((8, 128), F32)
        for b, xn in enumerate(normed):
            xn_ref[_span(i * nblk + b, R), :] = xn
            upd_ref[_span(i * nblk + b, R), :] = jnp.zeros((R, D), F32)
            r = jnp.sum(xn.astype(F32) * wr, axis=-1, keepdims=True)
            for j in range(R // 8):
                score = jnp.where(lane % per_part == b * (R // 8) + j, r[j * 8:(j + 1) * 8], score)
        score_ref[i] = score

    def first_step():
        halves = [slice(0, QW // 2), slice(QW // 2, QW)]
        pieces = [pltpu.make_async_copy(wq_hbm.at[:, c], wq_ref.at[0, :, c], h_sem.at[i])
                  for i, c in enumerate(halves)]
        _start([x_copies[0]] + pieces + [x_copies[1]])
        for ref in (wg_ref, wu_ref, wd_ref):
            ref[F:, :] = jnp.zeros((ref.shape[0] - F, D), BF16)
        xs_ref[...] = jnp.zeros_like(xs_ref)
        y_ref[...] = jnp.zeros_like(y_ref)
        x_copies[0].wait()
        normed = [_layernorm(x_ref[_span(b, R), :]) for b in range(EARLY)]
        pieces[0].wait()
        wq_copy(1).start()
        for b in range(EARLY):
            project_q(normed[b], 0, _span(b, R), halves[0])
        pieces[1].wait()
        for b in range(EARLY):
            if b == EARLY // 2:
                x_copies[1].wait()
                wr_copy.start()
            project_q(normed[b], 0, _span(b, R), halves[1])
        for b in range(EARLY, nblk):
            normed.append(_layernorm(x_ref[_span(b, R), :]))
            project_q(normed[b], 0, _span(b, R))
        _wait([wq_copy(1), wr_copy])
        wrf_ref[...] = wr_ref[...].astype(F32)
        _start(x_copies[2:])
        for b in range(nblk):
            project_q(normed[b], 1, _span(b, R))
        keep(0, normed)
        head_ref[...] = _layernorm(x_ref[_span(nblk, R), :])

    def norm_step(i):
        for j in range(1, norm_parts):
            pl.when(i == j)(x_copies[j + 1].wait)
        pl.when(i == 1)(functools.partial(_start, [wq_copy(2), wq_copy(3)] + ffn_copies))
        pl.when(i == norm_parts - 1)(functools.partial(_start, [wq_copy(j) for j in range(4, panels)]))
        normed, done = [head_ref[...]], []

        def pace(b):
            if b < 2:
                return None
            tiles = [divmod(3 + j, QW // 128) for j in range(R // 16)]
            return jnp.concatenate([done[2 * (b - 2) + d][j * 16:(j + 1) * 16, t * 128:(t + 1) * 128]
                                    for j, (d, t) in enumerate(tiles)], axis=0)

        for b in range(nblk):
            rows = _span(i * nblk + b, R)
            if b:
                normed.append(_layernorm(x_ref[rows, :], pace(b)))
            done.append(project_q(normed[b], 0, rows))
            done.append(project_q(normed[b], 1, rows))
        keep(i, normed)
        following = jnp.minimum(i + 1, norm_parts - 1) * nblk
        head_ref[...] = _layernorm(x_ref[_span(following, R), :], pace(nblk))

    def route():
        tiles, side = [], 128 // per_part
        for t in range(norm_parts // side):
            tile = score_ref[t * side]
            for j in range(1, side):
                tile = jnp.where(lane // per_part == j, score_ref[t * side + j], tile)
            tiles.append(tile)
        r = _bf(jnp.concatenate(tiles, axis=1))
        r = jnp.where(r == 0.0, 0.0, r)
        bits = pltpu.bitcast(r, I32) >> 16
        rank = jnp.where(r != r, 0, jnp.where(bits < 0, ~bits, bits + 0x8000))
        token = lax.broadcasted_iota(I32, r.shape, 1) * 8 + lax.broadcasted_iota(I32, r.shape, 0)
        key = pltpu.bitcast(((rank << 11) | (S - 1 - token)) + 0x08000000, F32)
        slot = lax.broadcasted_iota(I32, (CAP, 128), 0)
        top = jnp.zeros((CAP, 128), F32)
        for c in range(CAP):
            best = jnp.max(jnp.max(key, axis=0, keepdims=True), axis=1, keepdims=True)
            top = jnp.where(slot == c, best, top)
            key = jnp.where(key == best, 0.0, key)
        return pltpu.bitcast(top, I32) - 0x08000000

    def tokens(top):
        return [(S - 1) - (top[c, 0] & (S - 1)) for c in range(CAP)]

    def gather(top):
        row = lax.broadcasted_iota(I32, (16, D), 0)
        slot = lax.broadcasted_iota(I32, (CAP, D), 0)
        xs = jnp.zeros((CAP, D), F32)
        for c, t in enumerate(tokens(top)):
            near = xn_ref[_span(t >> 4, 16), :].astype(F32)
            xs = jnp.where(slot == c, jnp.sum(jnp.where(row == (t & 15), near, 0.0), axis=0, keepdims=True), xs)
        return xs

    def panel_step(i):
        pair, part = _divmod(i + proj_parts, proj_parts)

        hidden = _span(jnp.where(i == 0, wg_ref.shape[0] // FFN_CHUNK - 1, i - 1), FFN_CHUNK)
        xs = xs_ref[...]
        tiles = D // 128
        st = {}

        def swiglu(stage, k):
            cols = slice(k * 128, (k + 1) * 128)
            if stage < 2:
                t = lax.dot_general(xs[:, cols], (wg_ref, wu_ref)[stage][hidden, cols], NT, preferred_element_type=F32)
                st[stage] = t + st[stage] if k else t
            else:
                if k == 0:
                    st["h"] = _bf(_bf(_silu(_bf(st[0]))) * _bf(st[1]))
                st["y", k] = lax.dot_general(st["h"], wd_ref[hidden, cols], NN, preferred_element_type=F32)

        small = [(stage, k) for stage in range(3) for k in range(tiles)]
        small.insert(2 * tiles, None)
        assert len(small) == 2 * PROJ_ROWS // PROJ_BLOCK
        for b in range(PROJ_ROWS // PROJ_BLOCK):
            rows = _span(part * (PROJ_ROWS // PROJ_BLOCK) + b, PROJ_BLOCK)
            xn = xn_ref[rows, :]
            for half in range(2):
                project_q(xn, 2 * pair + half, rows)
                if small[2 * b + half]:
                    swiglu(*small[2 * b + half])
        top = route()
        top_ref[...] = top
        xs_ref[...] = gather(top)
        y_ref[...] += jnp.concatenate([st["y", k] for k in range(tiles)], axis=1)

    units, steps, per_panel = BLOCKS * HEADS, groups * parts, QW // DH

    def attention(i):
        after = min(i + 1, steps - 1) if isinstance(i, int) else jnp.minimum(i + 1, steps - 1)

        def place(u):
            b, h = divmod(u % units, HEADS)
            g, part = _divmod(i if u < units else after, parts)
            return g, _span(part * BLOCKS + b, R), h

        def query(u):
            g, rows, h = place(u)
            panel, col = divmod(h, per_panel)
            return q_ref[g * (HEADS // per_panel) + panel, rows, col * DH:(col + 1) * DH]

        def cache(ref, u, c):
            g, _, h = place(u)
            return ref[g * HEADS + h, c * CK:(c + 1) * CK, :]

        return _Attention(chunks, query, functools.partial(cache, k_ref), functools.partial(cache, v_ref))

    def hand_over(att, first):
        for j in range(AHEAD):
            s_ref[j] = att.s[first + j]
        m_ref[0] = _row_max(att.m[first // chunks])
        for u in range(1, pl.cdiv(AHEAD, chunks)):
            m_ref[u] = att.m[first // chunks + u]

    def project_o(o, g, h0, a):
        w = wo_ref[pl.ds(pl.multiple_of(g * (HEADS * DH), HEADS * DH) + h0 * DH, MERGE * DH), :]
        return jnp.dot(o, w, preferred_element_type=F32) + a

    def finish(rows, a):
        acc_ref[rows, :] = a
        gate = _silu(xn_ref[rows, :].astype(F32) + upd_ref[rows, :])
        out_ref[rows, :] = (x_ref[rows, :].astype(F32) + a * gate).astype(out_ref.dtype)

    def finish_step(step):
        g, part = _divmod(step, parts)
        o = _merge_heads([(tail_ref[0, h], tail_ref[1, h]) for h in range(MERGE)])
        finish(_span(part * BLOCKS + BLOCKS - 1, R), project_o(o, g, HEADS - MERGE, part_ref[...]))

    def prime():
        _wait(group_copies(0))
        _start([c for g in range(1, groups) for c in group_copies(g)])
        att = attention(0)
        for j in range(AHEAD):
            att.scores(j)
        hand_over(att, 0)
        tail_ref[...] = jnp.ones_like(tail_ref)
        part_ref[...] = jnp.zeros_like(part_ref)
        top = top_ref[...]
        rank = top >> 11
        r_sel = pltpu.bitcast(jnp.where(rank < 0x8000, ~rank, rank - 0x8000) << 16, F32)
        y = _bf(_bf(y_ref[...]) * _bf(jax.nn.sigmoid(r_sel[:, :1])))
        for c, t in enumerate(tokens(top)):
            upd_ref[pl.ds(t, 1), :] = y[c:c + 1, :]

    def attend_step(i):
        g, part = _divmod(i, parts)
        att = attention(i)
        for j in range(AHEAD):
            att.s[j] = s_ref[j]
        for u in range(pl.cdiv(AHEAD, chunks)):
            att.m[u] = m_ref[u]
        att.whole.add(0)
        acc = {}

        def project_heads(b, h0):
            rows, u0 = _span(part * BLOCKS + b, R), b * HEADS + h0
            a = acc[b] if h0 else jnp.where(g > 0, acc_ref[rows, :], 0.0)
            acc[b] = project_o(_merge_heads([(att.o[u], att.l[u]) for u in range(u0, u0 + MERGE)]), g, h0, a)
            if h0 + MERGE == HEADS:
                finish(rows, acc[b])

        program = [((LAG, 2), finish_step, (jnp.maximum(i - 1, 0),))]
        for j in range(units * chunks):
            program.append(((j, 0), att.values, (j,)))
            program.append(((j + AHEAD - LEAD, 1), att.scores, (j + AHEAD,)))
        for u in range(MERGE, units, MERGE):
            program.append(((u * chunks + LAG, 2), project_heads, divmod(u - MERGE, HEADS)))
        for _, fn, args in sorted(program, key=lambda e: e[0]):
            fn(*args)
        hand_over(att, units * chunks)
        for h in range(MERGE):
            tail_ref[0, h] = att.o[units - MERGE + h]
            tail_ref[1, h] = att.l[units - MERGE + h]
        part_ref[...] = acc[BLOCKS - 1]

        @pl.when(i > steps - parts)
        def _():
            out_copy(part - 1).start()

    @pl.loop(0, 2)
    def _(phase):
        @pl.when(phase == 0)
        def _():
            first_step()
            pl.loop(1, norm_parts)(norm_step)

        @pl.when(phase == 1)
        def _():
            _start(group_copies(0))
            _wait([wq_copy(2), wq_copy(3)])
            _loop_with_wait((panels // 2 - 1) * proj_parts, panel_step,
                            1, ffn_copies + [wq_copy(j) for j in range(4, panels)])
            prime()
            _loop_with_wait(steps, attend_step, parts - 1, [c for g in range(1, groups) for c in group_copies(g)])

    out_copy(parts - 1).start()
    finish_step(steps - 1)
    out_copy(parts).start()
    _wait([out_copy(p) for p in range(parts + 1)])


@jax.jit
def pallas_recurrent_scan__mha_block_cached__moe_arch_mod__prompt_kernel(
    A_x: jax.Array,
    A_k_cache: jax.Array,
    A_v_cache: jax.Array,
    A_wq: jax.Array,
    A_wo: jax.Array,
    B_x: jax.Array,
    B_w_r: jax.Array,
    B_w_gate: jax.Array,
    B_w_up: jax.Array,
    B_w_down: jax.Array,
):
    del B_x
    B, S, D = A_x.shape
    Sk = A_k_cache.shape[2]
    panels = H * DH // QW
    hidden = (panels // 2 - 1) * (S // PROJ_ROWS) * FFN_CHUNK
    assert B == 1 and S == 2048 and Sk % CK == 0 and B_w_gate.shape[1] <= hidden - FFN_CHUNK
    hbm = pl.BlockSpec(memory_space=pltpu.HBM)
    vmem, dma = pltpu.VMEM, pltpu.SemaphoreType.DMA
    scratch = [
        vmem((S, D), BF16), vmem((S, D), BF16), vmem((S, D), F32), vmem((S, D), F32), vmem((S, D), A_x.dtype),
        vmem((panels, S, QW), BF16), vmem((H, Sk, DH), BF16), vmem((H, Sk, DH), BF16),
        vmem((panels, D, QW), BF16), vmem((H * DH, D), BF16),
        vmem((hidden, D), BF16), vmem((hidden, D), BF16), vmem((hidden, D), BF16),
        vmem((AHEAD, R, CK), F32), vmem((pl.cdiv(AHEAD * CK, Sk), R, 128), F32),
        vmem((2, MERGE, R, DH), F32), vmem((R, D), F32), vmem((R, D), BF16), vmem((S // NORM_ROWS, 8, 128), F32),
        vmem((CAP, D), F32), vmem((CAP, D), F32), vmem((CAP, 128), I32), vmem((D,), BF16), vmem((D,), F32),
        dma((S // NORM_ROWS + 1,)), dma((2,)), dma((panels,)), dma((4,)), dma((H // HEADS, 3)),
        dma((S // (BLOCKS * R) + 1,)),
    ]
    return pl.pallas_call(
        _kernel,
        in_specs=[hbm] * 9,
        out_specs=hbm,
        out_shape=jax.ShapeDtypeStruct((B, S, D), A_x.dtype),
        scratch_shapes=scratch,
        compiler_params=pltpu.CompilerParams(
            vmem_limit_bytes=112 * 1024 * 1024, internal_scratch_in_bytes=64 * 1024),
    )(A_x, A_k_cache, A_v_cache, A_wq, A_wo, B_w_r, B_w_gate.T, B_w_up.T, B_w_down)
```

```python
import functools
import math

import jax
import jax.numpy as jnp
from jax import lax
import jax.experimental.pallas as pl
import jax.experimental.pallas.tpu as pltpu

F32 = jnp.float32
BF16 = jnp.bfloat16
I32 = jnp.int32
NN = (((1,), (0,)), ((), ()))
NT = (((1,), (1,)), ((), ()))

H, DH = 32, 128
CAP = 8
EPS = 1e-5

QW = 4 * DH
R = 64
NORM_ROWS = 512
EARLY = 5
PROJ_ROWS = 1024
PROJ_BLOCK = 128
FFN_CHUNK = 384
CK = 512
HEADS = 16
BLOCKS = 4
MERGE = 4
LEAD = 7
AHEAD = 8
LAG = 3


def _divmod(i, n):
    assert n & (n - 1) == 0
    return i >> (n.bit_length() - 1), i & (n - 1)


def _span(i, n):
    return pl.ds(i * n if isinstance(i, int) else pl.multiple_of(i * n, n), n)


def _start(copies):
    for c in copies:
        c.start()


def _wait(copies):
    for c in copies:
        c.wait()


def _loop_with_wait(n, body, at, copies):
    @pl.loop(0, 2)
    def _(half):
        pl.when(half == 1)(functools.partial(_wait, copies))
        pl.loop(half * at, jnp.where(half == 0, at, n))(body)


def _bf(x):
    return x.astype(BF16).astype(F32)


def _silu(x):
    h = 0.5 * x
    return h + h * jnp.tanh(h)


def _reciprocal(d):
    r = pl.reciprocal(d, approx=True)
    return r * (2.0 - d * r)


def _after(x, other):
    return jnp.where(other > jnp.inf, other, x)


def _layernorm(x, pace=None):
    d = x.shape[-1]
    x = x.astype(F32)
    if pace is not None:
        x = jnp.concatenate([_after(x[:, :128], pace), x[:, 128:]], axis=1)
    mu = jnp.sum(x, axis=-1, keepdims=True) * (1.0 / d)
    xc = x - mu
    var = jnp.sum(xc * xc, axis=-1, keepdims=True) * (1.0 / d)
    den = _bf(jnp.sqrt(_bf(_bf(var) + _bf(jnp.full_like(var, EPS)))))
    inv = jnp.where(den == jnp.inf, 0.0, _reciprocal(den))
    return (_bf(x - _bf(mu)) * inv).astype(BF16)


def _row_max(m):
    return jnp.broadcast_to(jnp.max(m, axis=-1, keepdims=True), m.shape)


class _Attention:
    def __init__(self, chunks, query, keys, vals):
        self.chunks, self.query, self.keys, self.vals = chunks, query, keys, vals
        self.q, self.s, self.m, self.l, self.o = {}, {}, {}, {}, {}
        self.whole = set()

    def scores(self, j):
        u, c = divmod(j, self.chunks)
        if u not in self.q:
            self.q[u] = self.query(u)
        s = self.s[j] = lax.dot_general(self.q[u], self.keys(u, c), NT, preferred_element_type=F32)
        m = jnp.maximum(s[:, :128], self.m[u]) if c else s[:, :128]
        for t in range(1, CK // 128):
            m = jnp.maximum(m, s[:, t * 128:(t + 1) * 128])
        self.m[u] = m

    def values(self, j):
        u, c = divmod(j, self.chunks)
        if c == 0 and u not in self.whole:
            self.m[u] = _row_max(self.m[u])
        p = jnp.exp2(self.s[j] - jnp.concatenate([self.m[u]] * (CK // 128), axis=1))
        l = p[:, :128] + self.l[u] if c else p[:, :128]
        for t in range(1, CK // 128):
            l = l + p[:, t * 128:(t + 1) * 128]
        self.l[u] = l
        p = jnp.concatenate([p[:, :-128], jnp.minimum(p[:, -128:], l)], axis=1)
        o = jnp.dot(p.astype(BF16), self.vals(u, c), preferred_element_type=F32)
        self.o[u] = o + self.o[u] if c else o


def _merge_heads(pairs):
    heads = [o * _reciprocal(jnp.sum(l, axis=-1, keepdims=True)) for o, l in pairs]
    return jnp.concatenate(heads, axis=1).astype(BF16)


def _kernel(x_hbm, k_hbm, v_hbm, wq_hbm, wo_hbm, wr_hbm, wg_hbm, wu_hbm, wd_hbm, out_hbm,
            x_ref, xn_ref, upd_ref, acc_ref, out_ref, q_ref, k_ref, v_ref, wq_ref, wo_ref,
            wg_ref, wu_ref, wd_ref, s_ref, m_ref, tail_ref, part_ref, head_ref, score_ref,
            xs_ref, y_ref, top_ref, wr_ref, wrf_ref,
            x_sem, h_sem, q_sem, w_sem, p_sem, o_sem):
    S, D = x_ref.shape
    F = wg_hbm.shape[0]
    panels, groups, chunks = H * DH // QW, H // HEADS, k_ref.shape[1] // CK
    norm_parts, proj_parts, parts = S // NORM_ROWS, S // PROJ_ROWS, S // (BLOCKS * R)
    qscale = (DH ** -0.5) * math.log2(math.e)

    edges = [0, EARLY * R] + [i * NORM_ROWS + R for i in range(1, norm_parts)] + [S]
    x_copies = [pltpu.make_async_copy(x_hbm.at[0, a:b], x_ref.at[a:b], x_sem.at[i])
                for i, (a, b) in enumerate(zip(edges, edges[1:]))]
    wr_copy = pltpu.make_async_copy(wr_hbm, wr_ref, w_sem.at[0])
    ffn_copies = [pltpu.make_async_copy(src, dst.at[:F], w_sem.at[i + 1])
                  for i, (src, dst) in enumerate([(wg_hbm, wg_ref), (wu_hbm, wu_ref), (wd_hbm, wd_ref)])]

    def wq_copy(i):
        return pltpu.make_async_copy(wq_hbm.at[:, _span(i, QW)], wq_ref.at[i], q_sem.at[i])

    def group_copies(g):
        heads, rows = _span(g, HEADS), _span(g, HEADS * DH)
        return [pltpu.make_async_copy(k_hbm.at[0, heads], k_ref.at[heads], p_sem.at[g, 0]),
                pltpu.make_async_copy(v_hbm.at[0, heads], v_ref.at[heads], p_sem.at[g, 1]),
                pltpu.make_async_copy(wo_hbm.at[rows], wo_ref.at[rows], p_sem.at[g, 2])]

    def out_copy(i):
        rows = _span(i, BLOCKS * R)
        if isinstance(i, int) and i >= parts - 1:
            rows = pl.ds(S - BLOCKS * R, (BLOCKS - 1) * R) if i < parts else pl.ds(S - R, R)
        return pltpu.make_async_copy(out_ref.at[rows], out_hbm.at[0, rows], o_sem.at[i])

    lane = lax.broadcasted_iota(I32, (8, 128), 1)
    per_part = NORM_ROWS // 8
    nblk = NORM_ROWS // R

    def project_q(xn, panel, rows, cols=slice(None)):
        q = jnp.dot(xn, wq_ref[panel, :, cols], preferred_element_type=F32)
        q_ref[panel, rows, cols] = (q * qscale).astype(BF16)
        return q

    def score_rows(i, normed):
        wr = wrf_ref[...].reshape(1, D)
        score = jnp.zeros((8, 128), F32)
        for b, xn in enumerate(normed):
            r = jnp.sum(xn.astype(F32) * wr, axis=-1, keepdims=True)
            for j in range(R // 8):
                score = jnp.where(lane % per_part == b * (R // 8) + j, r[j * 8:(j + 1) * 8], score)
        score_ref[i] = score

    def first_step():
        halves = [slice(0, QW // 2), slice(QW // 2, QW)]
        pieces = [pltpu.make_async_copy(wq_hbm.at[:, c], wq_ref.at[0, :, c], h_sem.at[i])
                  for i, c in enumerate(halves)]
        _start([x_copies[0]] + pieces + [x_copies[1]])
        for ref in (wg_ref, wu_ref, wd_ref):
            ref[F:, :] = jnp.zeros((ref.shape[0] - F, D), BF16)
        xs_ref[...] = jnp.zeros_like(xs_ref)
        y_ref[...] = jnp.zeros_like(y_ref)
        upd_ref[:NORM_ROWS, :] = jnp.zeros((NORM_ROWS, D), F32)
        x_copies[0].wait()
        normed = [_layernorm(x_ref[_span(b, R), :]) for b in range(EARLY)]
        for b in range(EARLY):
            xn_ref[_span(b, R), :] = normed[b]
        pieces[0].wait()
        wq_copy(1).start()
        for b in range(EARLY):
            project_q(normed[b], 0, _span(b, R), halves[0])
        pieces[1].wait()
        for b in range(EARLY):
            if b == EARLY // 2:
                x_copies[1].wait()
                wr_copy.start()
            project_q(normed[b], 0, _span(b, R), halves[1])
        for b in range(EARLY, nblk):
            normed.append(_layernorm(x_ref[_span(b, R), :]))
            project_q(normed[b], 0, _span(b, R))
            xn_ref[_span(b, R), :] = normed[b]
        _wait([wq_copy(1), wr_copy])
        wrf_ref[...] = wr_ref[...].astype(F32)
        _start(x_copies[2:])
        done = [project_q(normed[b], 1, _span(b, R)) for b in range(nblk)]
        score_rows(0, normed)
        head_ref[...] = _layernorm(x_ref[_span(nblk, R), :], done[3][:, :128])

    def norm_step(i):
        for j in range(1, norm_parts):
            pl.when(i == j)(x_copies[j + 1].wait)
        pl.when(i == 1)(functools.partial(_start, [wq_copy(2), wq_copy(3)] + ffn_copies))
        pl.when(i == norm_parts - 1)(functools.partial(_start, [wq_copy(j) for j in range(4, panels)]))
        normed, done = [head_ref[...]], []

        def pace(b):
            if b < 2:
                return None
            tiles = [divmod(3 + j, QW // 128) for j in range(R // 16)]
            return jnp.concatenate([done[2 * (b - 2) + d][j * 16:(j + 1) * 16, t * 128:(t + 1) * 128]
                                    for j, (d, t) in enumerate(tiles)], axis=0)

        for b in range(nblk):
            rows = _span(i * nblk + b, R)
            if b:
                normed.append(_layernorm(x_ref[rows, :], pace(b)))
            done.append(project_q(normed[b], 0, rows))
            done.append(project_q(normed[b], 1, rows))
        for b, xn in enumerate(normed):
            xn_ref[_span(i * nblk + b, R), :] = xn
            upd_ref[_span(i * nblk + b, R), :] = jnp.zeros((R, D), F32)
        score_rows(i, normed)
        following = jnp.minimum(i + 1, norm_parts - 1) * nblk
        head_ref[...] = _layernorm(x_ref[_span(following, R), :], pace(nblk))

    def route():
        tiles, side = [], 128 // per_part
        for t in range(norm_parts // side):
            tile = score_ref[t * side]
            for j in range(1, side):
                tile = jnp.where(lane // per_part == j, score_ref[t * side + j], tile)
            tiles.append(tile)
        r = _bf(jnp.concatenate(tiles, axis=1))
        r = jnp.where(r == 0.0, 0.0, r)
        bits = pltpu.bitcast(r, I32) >> 16
        rank = jnp.where(r != r, 0, jnp.where(bits < 0, ~bits, bits + 0x8000))
        token = lax.broadcasted_iota(I32, r.shape, 1) * 8 + lax.broadcasted_iota(I32, r.shape, 0)
        key = pltpu.bitcast(((rank << 11) | (S - 1 - token)) + 0x08000000, F32)
        slot = lax.broadcasted_iota(I32, (CAP, 128), 0)
        top = jnp.zeros((CAP, 128), F32)
        for c in range(CAP):
            best = jnp.max(jnp.max(key, axis=0, keepdims=True), axis=1, keepdims=True)
            top = jnp.where(slot == c, best, top)
            key = jnp.where(key == best, 0.0, key)
        return pltpu.bitcast(top, I32) - 0x08000000

    def tokens(top):
        return [(S - 1) - (top[c, 0] & (S - 1)) for c in range(CAP)]

    def gather(top):
        row = lax.broadcasted_iota(I32, (16, D), 0)
        slot = lax.broadcasted_iota(I32, (CAP, D), 0)
        xs = jnp.zeros((CAP, D), F32)
        for c, t in enumerate(tokens(top)):
            near = xn_ref[_span(t >> 4, 16), :].astype(F32)
            xs = jnp.where(slot == c, jnp.sum(jnp.where(row == (t & 15), near, 0.0), axis=0, keepdims=True), xs)
        return xs

    def panel_step(i):
        pair, part = _divmod(i + proj_parts, proj_parts)

        hidden = _span(jnp.where(i == 0, wg_ref.shape[0] // FFN_CHUNK - 1, i - 1), FFN_CHUNK)
        xs = xs_ref[...]
        tiles = D // 128
        st = {}

        def swiglu(stage, k):
            cols = slice(k * 128, (k + 1) * 128)
            if stage < 2:
                t = lax.dot_general(xs[:, cols], (wg_ref, wu_ref)[stage][hidden, cols], NT, preferred_element_type=F32)
                st[stage] = t + st[stage] if k else t
            else:
                if k == 0:
                    st["h"] = _bf(_bf(_silu(_bf(st[0]))) * _bf(st[1]))
                st["y", k] = lax.dot_general(st["h"], wd_ref[hidden, cols], NN, preferred_element_type=F32)

        small = [(stage, k) for stage in range(3) for k in range(tiles)]
        small.insert(2 * tiles, None)
        assert len(small) == 2 * PROJ_ROWS // PROJ_BLOCK
        for b in range(PROJ_ROWS // PROJ_BLOCK):
            rows = _span(part * (PROJ_ROWS // PROJ_BLOCK) + b, PROJ_BLOCK)
            xn = xn_ref[rows, :]
            for half in range(2):
                project_q(xn, 2 * pair + half, rows)
                if small[2 * b + half]:
                    swiglu(*small[2 * b + half])
        top = route()
        top_ref[...] = top
        xs_ref[...] = gather(top)
        y_ref[...] += jnp.concatenate([st["y", k] for k in range(tiles)], axis=1)

    units, steps, per_panel = BLOCKS * HEADS, groups * parts, QW // DH

    def attention(i):
        after = min(i + 1, steps - 1) if isinstance(i, int) else jnp.minimum(i + 1, steps - 1)

        def place(u):
            b, h = divmod(u % units, HEADS)
            g, part = _divmod(i if u < units else after, parts)
            return g, _span(part * BLOCKS + b, R), h

        def query(u):
            g, rows, h = place(u)
            panel, col = divmod(h, per_panel)
            return q_ref[g * (HEADS // per_panel) + panel, rows, col * DH:(col + 1) * DH]

        def cache(ref, u, c):
            g, _, h = place(u)
            return ref[g * HEADS + h, c * CK:(c + 1) * CK, :]

        return _Attention(chunks, query, functools.partial(cache, k_ref), functools.partial(cache, v_ref))

    def hand_over(att, first):
        for j in range(AHEAD):
            s_ref[j] = att.s[first + j]
        m_ref[0] = _row_max(att.m[first // chunks])
        for u in range(1, pl.cdiv(AHEAD, chunks)):
            m_ref[u] = att.m[first // chunks + u]

    def project_o(o, g, h0, a):
        w = wo_ref[pl.ds(pl.multiple_of(g * (HEADS * DH), HEADS * DH) + h0 * DH, MERGE * DH), :]
        return jnp.dot(o, w, preferred_element_type=F32) + a

    def finish(rows, a):
        acc_ref[rows, :] = a
        gate = _silu(xn_ref[rows, :].astype(F32) + upd_ref[rows, :])
        out_ref[rows, :] = (x_ref[rows, :].astype(F32) + a * gate).astype(out_ref.dtype)

    def finish_step(step):
        g, part = _divmod(step, parts)
        o = _merge_heads([(tail_ref[0, h], tail_ref[1, h]) for h in range(MERGE)])
        finish(_span(part * BLOCKS + BLOCKS - 1, R), project_o(o, g, HEADS - MERGE, part_ref[...]))

    def prime():
        _wait(group_copies(0))
        _start([c for g in range(1, groups) for c in group_copies(g)])
        att = attention(0)
        for j in range(AHEAD):
            att.scores(j)
        hand_over(att, 0)
        tail_ref[...] = jnp.ones_like(tail_ref)
        part_ref[...] = jnp.zeros_like(part_ref)
        top = top_ref[...]
        rank = top >> 11
        r_sel = pltpu.bitcast(jnp.where(rank < 0x8000, ~rank, rank - 0x8000) << 16, F32)
        y = _bf(_bf(y_ref[...]) * _bf(jax.nn.sigmoid(r_sel[:, :1])))
        for c, t in enumerate(tokens(top)):
            upd_ref[pl.ds(t, 1), :] = y[c:c + 1, :]

    def attend_step(i):
        g, part = _divmod(i, parts)
        att = attention(i)
        for j in range(AHEAD):
            att.s[j] = s_ref[j]
        for u in range(pl.cdiv(AHEAD, chunks)):
            att.m[u] = m_ref[u]
        att.whole.add(0)
        acc = {}

        def project_heads(b, h0):
            rows, u0 = _span(part * BLOCKS + b, R), b * HEADS + h0
            a = acc[b] if h0 else jnp.where(g > 0, acc_ref[rows, :], 0.0)
            acc[b] = project_o(_merge_heads([(att.o[u], att.l[u]) for u in range(u0, u0 + MERGE)]), g, h0, a)
            if h0 + MERGE == HEADS:
                finish(rows, acc[b])

        program = [((LAG, 2), finish_step, (jnp.maximum(i - 1, 0),))]
        for j in range(units * chunks):
            program.append(((j, 0), att.values, (j,)))
            program.append(((j + AHEAD - LEAD, 1), att.scores, (j + AHEAD,)))
        for u in range(MERGE, units, MERGE):
            program.append(((u * chunks + LAG, 2), project_heads, divmod(u - MERGE, HEADS)))
        for _, fn, args in sorted(program, key=lambda e: e[0]):
            fn(*args)
        hand_over(att, units * chunks)
        for h in range(MERGE):
            tail_ref[0, h] = att.o[units - MERGE + h]
            tail_ref[1, h] = att.l[units - MERGE + h]
        part_ref[...] = acc[BLOCKS - 1]

        @pl.when(i > steps - parts)
        def _():
            out_copy(part - 1).start()

    @pl.loop(0, 2)
    def _(phase):
        @pl.when(phase == 0)
        def _():
            first_step()
            pl.loop(1, norm_parts)(norm_step)

        @pl.when(phase == 1)
        def _():
            _start(group_copies(0))
            _wait([wq_copy(2), wq_copy(3)])
            _loop_with_wait((panels // 2 - 1) * proj_parts, panel_step,
                            1, ffn_copies + [wq_copy(j) for j in range(4, panels)])
            prime()
            _loop_with_wait(steps, attend_step, parts - 1, [c for g in range(1, groups) for c in group_copies(g)])

    out_copy(parts - 1).start()
    finish_step(steps - 1)
    out_copy(parts).start()
    _wait([out_copy(p) for p in range(parts + 1)])


@jax.jit
def pallas_recurrent_scan__mha_block_cached__moe_arch_mod__prompt_kernel(
    A_x: jax.Array,
    A_k_cache: jax.Array,
    A_v_cache: jax.Array,
    A_wq: jax.Array,
    A_wo: jax.Array,
    B_x: jax.Array,
    B_w_r: jax.Array,
    B_w_gate: jax.Array,
    B_w_up: jax.Array,
    B_w_down: jax.Array,
):
    del B_x
    B, S, D = A_x.shape
    Sk = A_k_cache.shape[2]
    panels = H * DH // QW
    hidden = (panels // 2 - 1) * (S // PROJ_ROWS) * FFN_CHUNK
    assert B == 1 and S == 2048 and Sk % CK == 0 and B_w_gate.shape[1] <= hidden - FFN_CHUNK
    hbm = pl.BlockSpec(memory_space=pltpu.HBM)
    vmem, dma = pltpu.VMEM, pltpu.SemaphoreType.DMA
    scratch = [
        vmem((S, D), BF16), vmem((S, D), BF16), vmem((S, D), F32), vmem((S, D), F32), vmem((S, D), A_x.dtype),
        vmem((panels, S, QW), BF16), vmem((H, Sk, DH), BF16), vmem((H, Sk, DH), BF16),
        vmem((panels, D, QW), BF16), vmem((H * DH, D), BF16),
        vmem((hidden, D), BF16), vmem((hidden, D), BF16), vmem((hidden, D), BF16),
        vmem((AHEAD, R, CK), F32), vmem((pl.cdiv(AHEAD * CK, Sk), R, 128), F32),
        vmem((2, MERGE, R, DH), F32), vmem((R, D), F32), vmem((R, D), BF16), vmem((S // NORM_ROWS, 8, 128), F32),
        vmem((CAP, D), F32), vmem((CAP, D), F32), vmem((CAP, 128), I32), vmem((D,), BF16), vmem((D,), F32),
        dma((S // NORM_ROWS + 1,)), dma((2,)), dma((panels,)), dma((4,)), dma((H // HEADS, 3)),
        dma((S // (BLOCKS * R) + 1,)),
    ]
    return pl.pallas_call(
        _kernel,
        in_specs=[hbm] * 9,
        out_specs=hbm,
        out_shape=jax.ShapeDtypeStruct((B, S, D), A_x.dtype),
        scratch_shapes=scratch,
        compiler_params=pltpu.CompilerParams(
            vmem_limit_bytes=112 * 1024 * 1024, internal_scratch_in_bytes=64 * 1024),
    )(A_x, A_k_cache, A_v_cache, A_wq, A_wo, B_w_r, B_w_gate.T, B_w_up.T, B_w_down)
```

```python
import functools
import math

import jax
import jax.numpy as jnp
from jax import lax
import jax.experimental.pallas as pl
import jax.experimental.pallas.tpu as pltpu

F32 = jnp.float32
BF16 = jnp.bfloat16
I32 = jnp.int32
NN = (((1,), (0,)), ((), ()))
NT = (((1,), (1,)), ((), ()))

H, DH = 32, 128
CAP = 8
EPS = 1e-5

QW = 4 * DH
R = 64
NORM_ROWS = 512
EARLY = 5
PROJ_ROWS = 1024
PROJ_BLOCK = 128
FFN_CHUNK = 384
CK = 512
HEADS = 16
BLOCKS = 4
MERGE = 4
LEAD = 7
AHEAD = 8
LAG = 3


def _divmod(i, n):
    assert n & (n - 1) == 0
    return i >> (n.bit_length() - 1), i & (n - 1)


def _span(i, n):
    return pl.ds(i * n if isinstance(i, int) else pl.multiple_of(i * n, n), n)


def _start(copies):
    for c in copies:
        c.start()


def _wait(copies):
    for c in copies:
        c.wait()


def _loop_with_wait(n, body, at, copies):
    @pl.loop(0, 2)
    def _(half):
        pl.when(half == 1)(functools.partial(_wait, copies))
        pl.loop(half * at, jnp.where(half == 0, at, n))(body)


def _bf(x):
    return x.astype(BF16).astype(F32)


def _silu(x):
    h = 0.5 * x
    return h + h * jnp.tanh(h)


def _reciprocal(d):
    r = pl.reciprocal(d, approx=True)
    return r * (2.0 - d * r)


def _after(x, other):
    return jnp.where(other > jnp.inf, other, x)


def _layernorm(x, pace=None):
    d = x.shape[-1]
    x = x.astype(F32)
    if pace is not None:
        x = jnp.concatenate([_after(x[:, :128], pace), x[:, 128:]], axis=1)
    mu = jnp.sum(x, axis=-1, keepdims=True) * (1.0 / d)
    xc = x - mu
    var = jnp.sum(xc * xc, axis=-1, keepdims=True) * (1.0 / d)
    den = _bf(jnp.sqrt(_bf(_bf(var) + _bf(jnp.full_like(var, EPS)))))
    inv = jnp.where(den == jnp.inf, 0.0, _reciprocal(den))
    return (_bf(x - _bf(mu)) * inv).astype(BF16)


def _row_max(m):
    return jnp.broadcast_to(jnp.max(m, axis=-1, keepdims=True), m.shape)


class _Attention:
    def __init__(self, chunks, query, keys, vals):
        self.chunks, self.query, self.keys, self.vals = chunks, query, keys, vals
        self.q, self.s, self.m, self.l, self.o = {}, {}, {}, {}, {}
        self.whole = set()

    def scores(self, j):
        u, c = divmod(j, self.chunks)
        if u not in self.q:
            self.q[u] = self.query(u)
        s = self.s[j] = lax.dot_general(self.q[u], self.keys(u, c), NT, preferred_element_type=F32)
        m = jnp.maximum(s[:, :128], self.m[u]) if c else s[:, :128]
        for t in range(1, CK // 128):
            m = jnp.maximum(m, s[:, t * 128:(t + 1) * 128])
        self.m[u] = m

    def values(self, j):
        u, c = divmod(j, self.chunks)
        if c == 0 and u not in self.whole:
            self.m[u] = _row_max(self.m[u])
        p = jnp.exp2(self.s[j] - jnp.concatenate([self.m[u]] * (CK // 128), axis=1))
        l = p[:, :128] + self.l[u] if c else p[:, :128]
        for t in range(1, CK // 128):
            l = l + p[:, t * 128:(t + 1) * 128]
        self.l[u] = l
        p = jnp.concatenate([p[:, :-128], jnp.minimum(p[:, -128:], l)], axis=1)
        o = jnp.dot(p.astype(BF16), self.vals(u, c), preferred_element_type=F32)
        self.o[u] = o + self.o[u] if c else o


def _merge_heads(pairs):
    heads = [o * _reciprocal(jnp.sum(l, axis=-1, keepdims=True)) for o, l in pairs]
    return jnp.concatenate(heads, axis=1).astype(BF16)


def _kernel(x_hbm, k_hbm, v_hbm, wq_hbm, wo_hbm, wr_hbm, wg_hbm, wu_hbm, wd_hbm, out_hbm,
            x_ref, xn_ref, upd_ref, acc_ref, out_ref, q_ref, k_ref, v_ref, wq_ref, wo_ref,
            wg_ref, wu_ref, wd_ref, s_ref, m_ref, tail_ref, part_ref, head_ref, score_ref,
            xs_ref, y_ref, top_ref, wr_ref, wrf_ref,
            x_sem, h_sem, q_sem, w_sem, p_sem, o_sem):
    S, D = x_ref.shape
    F = wg_hbm.shape[0]
    panels, groups, chunks = H * DH // QW, H // HEADS, k_ref.shape[1] // CK
    norm_parts, proj_parts, parts = S // NORM_ROWS, S // PROJ_ROWS, S // (BLOCKS * R)
    qscale = (DH ** -0.5) * math.log2(math.e)

    edges = [0, EARLY * R] + [i * NORM_ROWS + R for i in range(1, norm_parts)] + [S]
    x_copies = [pltpu.make_async_copy(x_hbm.at[0, a:b], x_ref.at[a:b], x_sem.at[i])
                for i, (a, b) in enumerate(zip(edges, edges[1:]))]
    wr_copy = pltpu.make_async_copy(wr_hbm, wr_ref, w_sem.at[0])
    ffn_copies = [pltpu.make_async_copy(src, dst.at[:F], w_sem.at[i + 1])
                  for i, (src, dst) in enumerate([(wg_hbm, wg_ref), (wu_hbm, wu_ref), (wd_hbm, wd_ref)])]

    def wq_copy(i):
        return pltpu.make_async_copy(wq_hbm.at[:, _span(i, QW)], wq_ref.at[i], q_sem.at[i])

    def group_copies(g):
        heads, rows = _span(g, HEADS), _span(g, HEADS * DH)
        return [pltpu.make_async_copy(k_hbm.at[0, heads], k_ref.at[heads], p_sem.at[g, 0]),
                pltpu.make_async_copy(v_hbm.at[0, heads], v_ref.at[heads], p_sem.at[g, 1]),
                pltpu.make_async_copy(wo_hbm.at[rows], wo_ref.at[rows], p_sem.at[g, 2])]

    def out_copy(i):
        rows = _span(i, BLOCKS * R)
        if isinstance(i, int) and i >= parts - 1:
            rows = pl.ds(S - BLOCKS * R, (BLOCKS - 1) * R) if i < parts else pl.ds(S - R, R)
        return pltpu.make_async_copy(out_ref.at[rows], out_hbm.at[0, rows], o_sem.at[i])

    lane = lax.broadcasted_iota(I32, (8, 128), 1)
    per_part = NORM_ROWS // 8
    nblk = NORM_ROWS // R

    def project_q(xn, panel, rows, cols=slice(None)):
        q = jnp.dot(xn, wq_ref[panel, :, cols], preferred_element_type=F32)
        q_ref[panel, rows, cols] = (q * qscale).astype(BF16)
        return q

    def score_rows(i, normed):
        wr = wrf_ref[...].reshape(1, D)
        score = jnp.zeros((8, 128), F32)
        for b, xn in enumerate(normed):
            r = jnp.sum(xn.astype(F32) * wr, axis=-1, keepdims=True)
            for j in range(R // 8):
                score = jnp.where(lane % per_part == b * (R // 8) + j, r[j * 8:(j + 1) * 8], score)
        score_ref[i] = score

    def first_step():
        halves = [slice(0, QW // 2), slice(QW // 2, QW)]
        pieces = [pltpu.make_async_copy(wq_hbm.at[:, c], wq_ref.at[0, :, c], h_sem.at[i])
                  for i, c in enumerate(halves)]
        _start([x_copies[0]] + pieces + [x_copies[1]])
        for ref in (wg_ref, wu_ref, wd_ref):
            ref[F:, :] = jnp.zeros((ref.shape[0] - F, D), BF16)
        xs_ref[...] = jnp.zeros_like(xs_ref)
        y_ref[...] = jnp.zeros_like(y_ref)
        upd_ref[:NORM_ROWS, :] = jnp.zeros((NORM_ROWS, D), F32)
        x_copies[0].wait()
        normed = [_layernorm(x_ref[_span(b, R), :]) for b in range(EARLY)]
        for b in range(EARLY):
            xn_ref[_span(b, R), :] = normed[b]
        pieces[0].wait()
        wq_copy(1).start()
        for b in range(EARLY):
            project_q(normed[b], 0, _span(b, R), halves[0])
        pieces[1].wait()
        for b in range(EARLY):
            if b == EARLY // 2:
                x_copies[1].wait()
                wr_copy.start()
            project_q(normed[b], 0, _span(b, R), halves[1])
        for b in range(EARLY, nblk):
            normed.append(_layernorm(x_ref[_span(b, R), :]))
            project_q(normed[b], 0, _span(b, R))
            xn_ref[_span(b, R), :] = normed[b]
        _wait([wq_copy(1), wr_copy])
        wrf_ref[...] = wr_ref[...].astype(F32)
        _start(x_copies[2:])
        done = [project_q(normed[b], 1, _span(b, R)) for b in range(nblk)]
        score_rows(0, normed)
        head_ref[...] = _layernorm(x_ref[_span(nblk, R), :], done[3][:, :128])

    def norm_step(i):
        for j in range(1, norm_parts):
            pl.when(i == j)(x_copies[j + 1].wait)
        pl.when(i == 1)(functools.partial(_start, [wq_copy(2), wq_copy(3)] + ffn_copies))
        pl.when(i == norm_parts - 1)(functools.partial(_start, [wq_copy(j) for j in range(4, panels)]))
        normed, done = [head_ref[...]], []

        def pace(b):
            if b < 2:
                return None
            tiles = [divmod(3 + j, QW // 128) for j in range(R // 16)]
            return jnp.concatenate([done[2 * (b - 2) + d][j * 16:(j + 1) * 16, t * 128:(t + 1) * 128]
                                    for j, (d, t) in enumerate(tiles)], axis=0)

        for b in range(nblk):
            rows = _span(i * nblk + b, R)
            if b:
                normed.append(_layernorm(x_ref[rows, :], pace(b)))
            done.append(project_q(normed[b], 0, rows))
            done.append(project_q(normed[b], 1, rows))
        for b, xn in enumerate(normed):
            xn_ref[_span(i * nblk + b, R), :] = xn
            upd_ref[_span(i * nblk + b, R), :] = jnp.zeros((R, D), F32)
        score_rows(i, normed)
        following = jnp.minimum(i + 1, norm_parts - 1) * nblk
        head_ref[...] = _layernorm(x_ref[_span(following, R), :], pace(nblk))

    def route():
        tiles, side = [], 128 // per_part
        for t in range(norm_parts // side):
            tile = score_ref[t * side]
            for j in range(1, side):
                tile = jnp.where(lane // per_part == j, score_ref[t * side + j], tile)
            tiles.append(tile)
        r = _bf(jnp.concatenate(tiles, axis=1))
        r = jnp.where(r == 0.0, 0.0, r)
        bits = pltpu.bitcast(r, I32) >> 16
        rank = jnp.where(r != r, 0, jnp.where(bits < 0, ~bits, bits + 0x8000))
        token = lax.broadcasted_iota(I32, r.shape, 1) * 8 + lax.broadcasted_iota(I32, r.shape, 0)
        key = pltpu.bitcast(((rank << 11) | (S - 1 - token)) + 0x08000000, F32)
        slot = lax.broadcasted_iota(I32, (CAP, 128), 0)
        top = jnp.zeros((CAP, 128), F32)
        for c in range(CAP):
            best = jnp.max(jnp.max(key, axis=0, keepdims=True), axis=1, keepdims=True)
            top = jnp.where(slot == c, best, top)
            key = jnp.where(key == best, 0.0, key)
        return pltpu.bitcast(top, I32) - 0x08000000

    def tokens(top):
        return [(S - 1) - (top[c, 0] & (S - 1)) for c in range(CAP)]

    def gather(top):
        row = lax.broadcasted_iota(I32, (16, D), 0)
        slot = lax.broadcasted_iota(I32, (CAP, D), 0)
        xs = jnp.zeros((CAP, D), F32)
        for c, t in enumerate(tokens(top)):
            near = xn_ref[_span(t >> 4, 16), :].astype(F32)
            xs = jnp.where(slot == c, jnp.sum(jnp.where(row == (t & 15), near, 0.0), axis=0, keepdims=True), xs)
        return xs

    def panel_step(i):
        pair, part = _divmod(i + proj_parts, proj_parts)

        hidden = _span(jnp.where(i == 0, wg_ref.shape[0] // FFN_CHUNK - 1, i - 1), FFN_CHUNK)
        xs = xs_ref[...]
        tiles = D // 128
        st = {}

        def swiglu(stage, k):
            cols = slice(k * 128, (k + 1) * 128)
            if stage < 2:
                t = lax.dot_general(xs[:, cols], (wg_ref, wu_ref)[stage][hidden, cols], NT, preferred_element_type=F32)
                st[stage] = t + st[stage] if k else t
            else:
                if k == 0:
                    st["h"] = _bf(_bf(_silu(_bf(st[0]))) * _bf(st[1]))
                st["y", k] = lax.dot_general(st["h"], wd_ref[hidden, cols], NN, preferred_element_type=F32)

        small = [(stage, k) for stage in range(3) for k in range(tiles)]
        small.insert(2 * tiles, None)
        assert len(small) == 2 * PROJ_ROWS // PROJ_BLOCK
        for b in range(PROJ_ROWS // PROJ_BLOCK):
            rows = _span(part * (PROJ_ROWS // PROJ_BLOCK) + b, PROJ_BLOCK)
            xn = xn_ref[rows, :]
            for half in range(2):
                project_q(xn, 2 * pair + half, rows)
                if small[2 * b + half]:
                    swiglu(*small[2 * b + half])
        top = route()
        top_ref[...] = top
        xs_ref[...] = gather(top)
        y_ref[...] += jnp.concatenate([st["y", k] for k in range(tiles)], axis=1)

    units, steps, per_panel = BLOCKS * HEADS, groups * parts, QW // DH

    def attention(i):
        after = min(i + 1, steps - 1) if isinstance(i, int) else jnp.minimum(i + 1, steps - 1)

        def place(u):
            b, h = divmod(u % units, HEADS)
            g, part = _divmod(i if u < units else after, parts)
            return g, _span(part * BLOCKS + b, R), h

        def query(u):
            g, rows, h = place(u)
            panel, col = divmod(h, per_panel)
            return q_ref[g * (HEADS // per_panel) + panel, rows, col * DH:(col + 1) * DH]

        def cache(ref, u, c):
            g, _, h = place(u)
            return ref[g * HEADS + h, c * CK:(c + 1) * CK, :]

        return _Attention(chunks, query, functools.partial(cache, k_ref), functools.partial(cache, v_ref))

    def hand_over(att, first):
        for j in range(AHEAD):
            s_ref[j] = att.s[first + j]
        m_ref[0] = _row_max(att.m[first // chunks])
        for u in range(1, pl.cdiv(AHEAD, chunks)):
            m_ref[u] = att.m[first // chunks + u]

    def project_o(o, g, h0, a):
        w = wo_ref[pl.ds(pl.multiple_of(g * (HEADS * DH), HEADS * DH) + h0 * DH, o.shape[1]), :]
        return jnp.dot(o, w, preferred_element_type=F32) + a

    def finish(rows, a):
        acc_ref[rows, :] = a
        gate = _silu(xn_ref[rows, :].astype(F32) + upd_ref[rows, :])
        out_ref[rows, :] = (x_ref[rows, :].astype(F32) + a * gate).astype(out_ref.dtype)

    def finish_step(step):
        g, part = _divmod(step, parts)
        o = _merge_heads([(tail_ref[0], tail_ref[1])])
        finish(_span(part * BLOCKS + BLOCKS - 1, R), project_o(o, g, HEADS - 1, part_ref[...]))

    def prime():
        _wait(group_copies(0))
        _start([c for g in range(1, groups) for c in group_copies(g)])
        att = attention(0)
        for j in range(AHEAD):
            att.scores(j)
        hand_over(att, 0)
        tail_ref[...] = jnp.ones_like(tail_ref)
        part_ref[...] = jnp.zeros_like(part_ref)
        top = top_ref[...]
        rank = top >> 11
        r_sel = pltpu.bitcast(jnp.where(rank < 0x8000, ~rank, rank - 0x8000) << 16, F32)
        y = _bf(_bf(y_ref[...]) * _bf(jax.nn.sigmoid(r_sel[:, :1])))
        for c, t in enumerate(tokens(top)):
            upd_ref[pl.ds(t, 1), :] = y[c:c + 1, :]

    def attend_step(i):
        g, part = _divmod(i, parts)
        att = attention(i)
        for j in range(AHEAD):
            att.s[j] = s_ref[j]
        for u in range(pl.cdiv(AHEAD, chunks)):
            att.m[u] = m_ref[u]
        att.whole.add(0)
        acc = {}

        def project_heads(b, h0, n):
            rows, u0 = _span(part * BLOCKS + b, R), b * HEADS + h0
            a = acc[b] if h0 else jnp.where(g > 0, acc_ref[rows, :], 0.0)
            acc[b] = project_o(_merge_heads([(att.o[u], att.l[u]) for u in range(u0, u0 + n)]), g, h0, a)
            if h0 + n == HEADS:
                finish(rows, acc[b])

        program = [((LAG, 2), finish_step, (jnp.maximum(i - 1, 0),))]
        for j in range(units * chunks):
            program.append(((j, 0), att.values, (j,)))
            program.append(((j + AHEAD - LEAD, 1), att.scores, (j + AHEAD,)))
        cuts = list(range(0, units, MERGE)) + [units - 1]
        for u0, u1 in zip(cuts, cuts[1:]):
            program.append(((u1 * chunks + LAG, 2), project_heads, divmod(u0, HEADS) + (u1 - u0,)))
        for _, fn, args in sorted(program, key=lambda e: e[0]):
            fn(*args)
        hand_over(att, units * chunks)
        tail_ref[0], tail_ref[1] = att.o[units - 1], att.l[units - 1]
        part_ref[...] = acc[BLOCKS - 1]

        @pl.when(i > steps - parts)
        def _():
            out_copy(part - 1).start()

    @pl.loop(0, 2)
    def _(phase):
        @pl.when(phase == 0)
        def _():
            first_step()
            pl.loop(1, norm_parts)(norm_step)

        @pl.when(phase == 1)
        def _():
            _start(group_copies(0))
            _wait([wq_copy(2), wq_copy(3)])
            _loop_with_wait((panels // 2 - 1) * proj_parts, panel_step,
                            1, ffn_copies + [wq_copy(j) for j in range(4, panels)])
            prime()
            _loop_with_wait(steps, attend_step, parts - 1, [c for g in range(1, groups) for c in group_copies(g)])

    out_copy(parts - 1).start()
    finish_step(steps - 1)
    out_copy(parts).start()
    _wait([out_copy(p) for p in range(parts + 1)])


@jax.jit
def pallas_recurrent_scan__mha_block_cached__moe_arch_mod__prompt_kernel(
    A_x: jax.Array,
    A_k_cache: jax.Array,
    A_v_cache: jax.Array,
    A_wq: jax.Array,
    A_wo: jax.Array,
    B_x: jax.Array,
    B_w_r: jax.Array,
    B_w_gate: jax.Array,
    B_w_up: jax.Array,
    B_w_down: jax.Array,
):
    del B_x
    B, S, D = A_x.shape
    Sk = A_k_cache.shape[2]
    panels = H * DH // QW
    hidden = (panels // 2 - 1) * (S // PROJ_ROWS) * FFN_CHUNK
    assert B == 1 and S == 2048 and Sk % CK == 0 and B_w_gate.shape[1] <= hidden - FFN_CHUNK
    hbm = pl.BlockSpec(memory_space=pltpu.HBM)
    vmem, dma = pltpu.VMEM, pltpu.SemaphoreType.DMA
    scratch = [
        vmem((S, D), BF16), vmem((S, D), BF16), vmem((S, D), F32), vmem((S, D), F32), vmem((S, D), A_x.dtype),
        vmem((panels, S, QW), BF16), vmem((H, Sk, DH), BF16), vmem((H, Sk, DH), BF16),
        vmem((panels, D, QW), BF16), vmem((H * DH, D), BF16),
        vmem((hidden, D), BF16), vmem((hidden, D), BF16), vmem((hidden, D), BF16),
        vmem((AHEAD, R, CK), F32), vmem((pl.cdiv(AHEAD * CK, Sk), R, 128), F32),
        vmem((2, R, DH), F32), vmem((R, D), F32), vmem((R, D), BF16), vmem((S // NORM_ROWS, 8, 128), F32),
        vmem((CAP, D), F32), vmem((CAP, D), F32), vmem((CAP, 128), I32), vmem((D,), BF16), vmem((D,), F32),
        dma((S // NORM_ROWS + 1,)), dma((2,)), dma((panels,)), dma((4,)), dma((H // HEADS, 3)),
        dma((S // (BLOCKS * R) + 1,)),
    ]
    return pl.pallas_call(
        _kernel,
        in_specs=[hbm] * 9,
        out_specs=hbm,
        out_shape=jax.ShapeDtypeStruct((B, S, D), A_x.dtype),
        scratch_shapes=scratch,
        compiler_params=pltpu.CompilerParams(
            vmem_limit_bytes=112 * 1024 * 1024, internal_scratch_in_bytes=64 * 1024),
    )(A_x, A_k_cache, A_v_cache, A_wq, A_wo, B_w_r, B_w_gate.T, B_w_up.T, B_w_down)
```
